```python
import os as _os
_os.environ.setdefault("JAX_PLATFORMS", "cpu")
import jax
import jax.numpy as jnp

def _softmax(x, axis=-1):
    return jax.nn.softmax(x, axis=axis)
def _gelu(x):
    return jax.nn.gelu(x, approximate=True)
def _silu(x):
    return jax.nn.silu(x)
def _sigmoid(x):
    return jax.nn.sigmoid(x)
def _layernorm(x, axis=-1, eps=1e-5):
    m = jnp.mean(x, axis=axis, keepdims=True)
    v = jnp.var(x, axis=axis, keepdims=True)
    return (x - m) / jnp.sqrt(v + eps)
def _scatter_add(tgt, idx, src, axis=0):
    return tgt.at[idx].add(src)
def _segment_sum(src, seg, n):
    return jax.ops.segment_sum(src, seg, n)
class _Rng:
    def __init__(self, key):
        self._k = key
    def _next(self):
        self._k, sub = jax.random.split(self._k)
        return sub
    def normal(self, shape):
        return jax.random.normal(self._next(), shape, dtype=jnp.bfloat16)
    def randint(self, lo, hi, shape):
        return jax.random.randint(self._next(), shape, lo, hi, dtype=jnp.int32)
    def uniform(self, shape, lo=0.0, hi=1.0):
        return jax.random.uniform(self._next(), shape, jnp.bfloat16, lo, hi)
    def permutation(self, n):
        return jax.random.permutation(self._next(), n)


kernel_name = 'parallel_sum__grouped_kv_mqa__dense_activation_silu__prompt'

def setup_inputs():
    _rng = _Rng(jax.random.key(int.from_bytes(__import__("os").urandom(4), "little")))
    _w = (lambda a: (lambda t: t.astype(jnp.bfloat16) if jnp.issubdtype(t.dtype, jnp.floating) else t)(jnp.asarray(a)))
    def _A_setup():
        B, S, D, H = 1, 2048, 512, 32
        Dh = D // H
        return {
            "x": _w((lambda *s: _rng.normal(s) * 0.05)(B, S, D)),
            "wq": _w((lambda *s: _rng.normal(s) * 0.05)(D, H * Dh)),
            "wk": _w((lambda *s: _rng.normal(s) * 0.05)(D, Dh)),
            "wv": _w((lambda *s: _rng.normal(s) * 0.05)(D, Dh)),
            "wo": _w((lambda *s: _rng.normal(s) * 0.05)(H * Dh, D)),
        }
    _A_in = _A_setup()

    def _B_setup():
        B, S, D, F = 1, 2048, 512, 1376
        return {
            "x": _w((lambda *s: _rng.normal(s) * 0.05)(B, S, D)),
            "w1": _w((lambda *s: _rng.normal(s) * 0.05)(D, F) * (D ** -0.5)),
            "w2": _w((lambda *s: _rng.normal(s) * 0.05)(F, D) * (F ** -0.5)),
        }
    _B_in = _B_setup()

    return {
        "A_x": _A_in["x"],
        "A_wq": _A_in["wq"],
        "A_wk": _A_in["wk"],
        "A_wv": _A_in["wv"],
        "A_wo": _A_in["wo"],
        "B_x": _B_in["x"],
        "B_w1": _B_in["w1"],
        "B_w2": _B_in["w2"],
    }

def reference(A_x, A_wq, A_wk, A_wv, A_wo, B_x, B_w1, B_w2):
    def _A_ref(x, wq, wk, wv, wo):
        B, S, D = x.shape
        H = 32
        Dh = D // H
        q = (lambda x, *d: x.transpose(*d))((x @ wq).reshape(B, S, H, Dh), 0, 2, 1, 3)
        k = x @ wk
        v = x @ wv
        scores = jnp.einsum("bhqd,bkd->bhqk", q, k) * (Dh ** -0.5)
        p = _softmax(scores, axis=-1)
        o = jnp.einsum("bhqk,bkd->bhqd", p, v)
        return (lambda x, *d: x.transpose(*d))(o, 0, 2, 1, 3).reshape(B, S, H * Dh) @ wo

    def _B_ref(x, w1, w2):
        h = jnp.einsum("bsd,df->bsf", x, w1)
        h = _silu(h)
        out = jnp.einsum("bsf,fd->bsd", h, w2)
        return out

    x = A_x
    xn = _layernorm(x, axis=-1)
    return x + _A_ref(xn, A_wq, A_wk, A_wv, A_wo) + _B_ref(xn, B_w1, B_w2)
```

```python
import functools
import math

import jax
import jax.numpy as jnp
import jax.experimental.pallas as pl
import jax.experimental.pallas.tpu as pltpu

_H = 32
_EPS = 1e-5
_TQ = 512
_CK = 128


def _kernel(x_ref, wq_ref, wk_ref, wv_ref, wo_ref, w1_ref, w2_ref, o_ref,
            xn_ref, qt_ref, k_ref, vt_ref, ot_ref, s_ref, *, S, D, Dh):
    f32, bf16 = jnp.float32, jnp.bfloat16
    H, TQ, CK = _H, _TQ, _CK
    NQ, NC = S // TQ, S // CK
    qscale = (Dh ** -0.5) * math.log2(math.e)

    def proj(i, _):
        r = pl.multiple_of(i * TQ, TQ)
        x = x_ref[pl.ds(r, TQ), :].astype(f32)
        mu = jnp.mean(x, axis=-1, keepdims=True)
        xc = x - mu
        var = jnp.mean(xc * xc, axis=-1, keepdims=True)
        xn = (xc * jax.lax.rsqrt(var + _EPS)).astype(bf16)
        xn_ref[pl.ds(r, TQ), :] = xn
        tn = (((0,), (1,)), ((), ()))
        qt = jax.lax.dot_general(wq_ref[...], xn, tn, preferred_element_type=f32)
        qt_ref[:, pl.ds(r, TQ)] = (qt * qscale).astype(bf16)
        vt = jax.lax.dot_general(wv_ref[...], xn, tn, preferred_element_type=f32)
        vt_ref[:, pl.ds(r, TQ)] = vt.astype(bf16)
        k = jnp.dot(xn, wk_ref[...], preferred_element_type=f32)
        k_ref[pl.ds(r, TQ), :] = k.astype(bf16)
        return 0

    jax.lax.fori_loop(0, NQ, proj, 0)

    def load_qt(u):
        h = u % H
        j = u // H
        return qt_ref[pl.ds(pl.multiple_of(h * Dh, Dh), Dh),
                      pl.ds(pl.multiple_of(j * TQ, TQ), TQ)]

    def scores_chunk(c, qt, mx):
        s = jnp.dot(k_ref[pl.ds(c * CK, CK), :], qt, preferred_element_type=f32)
        s_ref[pl.ds(c * CK, CK), :] = s
        return jnp.maximum(mx, jnp.max(s.reshape(CK // 8, 8, TQ), axis=0))

    def softmax_chunk(c, m, l, acc):
        p = jnp.exp2(s_ref[pl.ds(c * CK, CK), :] - m)
        l = l + jnp.sum(p.reshape(CK // 8, 8, TQ), axis=0)
        acc = acc + jnp.dot(vt_ref[:, pl.ds(c * CK, CK)], p.astype(bf16),
                            preferred_element_type=f32)
        return l, acc

    neg = jnp.full((8, TQ), -jnp.inf, f32)
    qt0 = load_qt(0)
    mx0 = neg
    for c in range(NC):
        mx0 = scores_chunk(c, qt0, mx0)

    NU = NQ * H

    def unit(u, mx):
        m = jnp.max(mx, axis=0, keepdims=True)
        qt = load_qt(jnp.minimum(u + 1, NU - 1))
        l = jnp.zeros((8, TQ), f32)
        acc = jnp.zeros((Dh, TQ), f32)
        mxn = neg
        for c in range(NC):
            l, acc = softmax_chunk(c, m, l, acc)
            mxn = scores_chunk(c, qt, mxn)
        lsum = jnp.sum(l, axis=0, keepdims=True)
        h = u % H
        j = u // H
        ot_ref[pl.ds(pl.multiple_of(h * Dh, Dh), Dh),
               pl.ds(pl.multiple_of(j * TQ, TQ), TQ)] = (acc / lsum).astype(bf16)
        return mxn

    jax.lax.fori_loop(0, NU, unit, mx0)

    def tail(i, _):
        r = pl.multiple_of(i * TQ, TQ)
        xn = xn_ref[pl.ds(r, TQ), :]
        attn = jax.lax.dot_general(ot_ref[:, pl.ds(r, TQ)], wo_ref[...],
                                   (((0,), (0,)), ((), ())), preferred_element_type=f32)
        hmid = jnp.dot(xn, w1_ref[...], preferred_element_type=f32)
        hmid = (hmid * jax.nn.sigmoid(hmid)).astype(bf16)
        ffn = jnp.dot(hmid, w2_ref[...], preferred_element_type=f32)
        o_ref[pl.ds(r, TQ), :] = (x_ref[pl.ds(r, TQ), :].astype(f32) + attn + ffn).astype(o_ref.dtype)
        return 0

    jax.lax.fori_loop(0, NQ, tail, 0)


@jax.jit
def pallas_parallel_sum__grouped_kv_mqa__dense_activation_silu__prompt_kernel(
    A_x: jax.Array,
    A_wq: jax.Array,
    A_wk: jax.Array,
    A_wv: jax.Array,
    A_wo: jax.Array,
    B_x: jax.Array,
    B_w1: jax.Array,
    B_w2: jax.Array,
):
    del B_x
    B, S, D = A_x.shape
    assert B == 1
    Dh = D // _H
    x = A_x.reshape(S, D)
    bf16 = jnp.bfloat16

    out = pl.pallas_call(
        functools.partial(_kernel, S=S, D=D, Dh=Dh),
        out_shape=jax.ShapeDtypeStruct((S, D), A_x.dtype),
        scratch_shapes=[
            pltpu.VMEM((S, D), bf16),
            pltpu.VMEM((D, S), bf16),
            pltpu.VMEM((S, Dh), bf16),
            pltpu.VMEM((Dh, S), bf16),
            pltpu.VMEM((D, S), bf16),
            pltpu.VMEM((S, _TQ), jnp.float32),
        ],
        compiler_params=pltpu.CompilerParams(vmem_limit_bytes=100 * 1024 * 1024),
    )(x, A_wq, A_wk, A_wv, A_wo, B_w1, B_w2)
    return out.reshape(B, S, D)
```

```python
import functools
import math

import jax
import jax.numpy as jnp
import jax.experimental.pallas as pl
import jax.experimental.pallas.tpu as pltpu

_H = 32
_EPS = 1e-5
_TQ = 512
_CK = 128
_GR = 16
_NG = _CK // _GR
_NMG = _NG - 1
_POS = (0, 2, 4, 6)
_UN = 4
_OFF = 1

_L_MIN = 2.0 ** -80
_L_MAX = 2.0 ** 60
_V_MAX = 2.0 ** 60


def _order(pos):
    o = list(range(_NMG))
    o.insert(pos, _NMG)
    return o


def _kernel(x_ref, wq_ref, wkt_ref, wvt_ref, wo_ref, w1t_ref, w2_ref, o_ref,
            xn_ref, wqt_ref, qt_ref, kv_ref, km_ref, kb_ref, vt_ref, vtp_ref,
            qb_ref, ot_ref, l_ref, *, S, D, Dh):
    f32, bf16 = jnp.float32, jnp.bfloat16
    H, TQ, CK, GR, NMG, UN = _H, _TQ, _CK, _GR, _NMG, _UN
    NQ, NC, J = S // TQ, S // CK, TQ // 128
    NU = NQ * H
    qscale = (Dh ** -0.5) * math.log2(math.e)
    nt = (((1,), (1,)), ((), ()))

    wqt_ref[...] = wq_ref[...].T
    wkvt = jnp.concatenate([wkt_ref[...], wvt_ref[...]], axis=0)

    def proj(i, _):
        r = pl.multiple_of(i * TQ, TQ)
        x = x_ref[pl.ds(r, TQ), :].astype(f32)
        mu = jnp.mean(x, axis=-1, keepdims=True)
        xc = x - mu
        var = jnp.mean(xc * xc, axis=-1, keepdims=True)
        xn = (xc * jax.lax.rsqrt(var + _EPS)).astype(bf16)
        xn_ref[pl.ds(r, TQ), :] = xn
        qt = jax.lax.dot_general(wqt_ref[...], xn, nt, preferred_element_type=f32)
        qt_ref[:, pl.ds(r, TQ)] = (qt * qscale).astype(bf16)
        kv = jax.lax.dot_general(xn, wkvt, nt, preferred_element_type=f32)
        kv_ref[pl.ds(r, TQ), :] = kv.astype(bf16)
        return 0

    jax.lax.fori_loop(0, NQ, proj, 0)

    row = jax.lax.broadcasted_iota(jnp.int32, (Dh, 2 * Dh), 0)
    col = jax.lax.broadcasted_iota(jnp.int32, (Dh, 2 * Dh), 1)
    sel = (col == row + Dh).astype(bf16)
    vt = jax.lax.dot_general(sel, kv_ref[...], nt, preferred_element_type=f32)
    vt_ref[...] = vt.astype(bf16)
    vmax = jnp.max(jnp.abs(vt))
    for j in range(J):
        for c in range(NC):
            rows = jnp.concatenate(
                [kv_ref[pl.ds(c * CK + g * GR, GR), :] for g in reversed(_order(_POS[j]))], axis=0)
            vtp_ref[j, :, pl.ds(c * CK, CK)] = jax.lax.dot_general(
                sel, rows, nt, preferred_element_type=f32).astype(bf16)
    for c in range(NC):
        km_ref[pl.ds(c * NMG * GR, NMG * GR), :] = kv_ref[pl.ds(c * CK, NMG * GR), :][:, :Dh]
        kf = kv_ref[pl.ds(c * CK + NMG * GR, GR), :].astype(f32)
        for d in range(Dh):
            kb_ref[d, pl.ds(c * GR, GR), :] = jnp.broadcast_to(kf[:, d:d + 1], (GR, 128))

    def unit_slices(u):
        h = u % H
        j = u // H
        return (pl.ds(pl.multiple_of(h * Dh, Dh), Dh), pl.ds(pl.multiple_of(j * TQ, TQ), TQ), h)

    def fast(i, _):
        zs = {(t, j): (i + t * J + j) // (1 << 20) for t in range(UN) for j in range(J)}
        sts, qts, srows = {}, {}, {}
        per_unit = NC * NMG
        total = UN * per_unit

        def start(t):
            rs, cs, _h = unit_slices(i * UN + t)
            qts[t] = qt_ref[rs, cs]
            qf = qts[t].astype(f32)
            for d in range(Dh):
                qb_ref[t, d] = jnp.broadcast_to(qf[d:d + 1, :], (8, TQ))
            sts[t] = dict(l=[jnp.zeros((8, 128), f32)] * J, acc=[jnp.zeros((Dh, 128), f32)] * J)

        def finish(t):
            rs, cs, h = unit_slices(i * UN + t)
            lsum = jnp.sum(jnp.concatenate(sts[t]['l'], axis=1), axis=0, keepdims=True)
            l_ref[pl.ds(h, 1), cs] = lsum
            ot_ref[rs, cs] = (jnp.concatenate(sts[t]['acc'], axis=1) / lsum).astype(bf16)

        def mxu_scores(a, b):
            while a < b:
                t = a // per_unit
                e = min(b, (t + 1) * per_unit)
                if t not in qts:
                    start(t)
                la, le = a - t * per_unit, e - t * per_unit
                kk = km_ref[pl.ds(la * GR, (le - la) * GR), :]
                for j in range(J):
                    s = jnp.dot(kk, qts[t][:, j * 128:(j + 1) * 128], preferred_element_type=f32)
                    for xg in range(la, le):
                        r = srows.setdefault((t, xg // NMG, j), [None] * (2 * _NG))
                        g, o = xg % NMG, (xg - la) * GR
                        r[2 * g] = s[o:o + 8, :]
                        r[2 * g + 1] = s[o + 8:o + 16, :]
                a = e

        def vpu_scores(t, c, j):
            acc = [None, None]
            for d in range(Dh):
                qb = qb_ref[t, d, :, pl.ds(j * 128, 128)]
                for half in range(2):
                    y = kb_ref[d + zs[(t, j)], pl.ds(c * GR + 8 * half, 8), :] * qb
                    acc[half] = y if d == 0 else acc[half] + y
            return acc

        def pv(t, c, j, rows):
            st, order = sts[t], _order(_POS[j])
            ps = {}
            for g in order:
                ps[2 * g] = jnp.exp2(rows[2 * g])
                ps[2 * g + 1] = jnp.exp2(rows[2 * g + 1])
            lc = ps[0]
            for r in range(1, 2 * _NG):
                lc = lc + ps[r]
            st['l'][j] = st['l'][j] + lc
            grp = []
            for g in reversed(order):
                grp += [ps[2 * g], ps[2 * g + 1]]
            p = jnp.concatenate(grp, axis=0).astype(bf16)
            st['acc'][j] = st['acc'][j] + jnp.dot(vtp_ref[j, :, pl.ds(c * CK, CK)], p,
                                                  preferred_element_type=f32)

        mxu_scores(0, NMG)
        done = NMG
        for t in range(UN):
            for c in range(NC):
                need = min(total, (t * NC + c + 2) * NMG + _OFF)
                mxu_scores(done, need)
                done = need
                for j in range(J):
                    r = srows.pop((t, c, j))
                    r[2 * NMG], r[2 * NMG + 1] = vpu_scores(t, c, j)
                    pv(t, c, j, r)
                if c == NC - 1:
                    finish(t)
        return 0

    jax.lax.fori_loop(0, NU // UN, fast, 0)

    lall = l_ref[...]
    l_ok = jnp.logical_and(lall >= _L_MIN, lall <= _L_MAX)
    n_bad = jnp.sum(jnp.where(l_ok, 0.0, 1.0))
    safe = jnp.logical_and(n_bad == 0.0, vmax <= _V_MAX)

    @pl.when(jnp.logical_not(safe))
    def _():
        def exact(u, _):
            rs, cs, _h = unit_slices(u)
            s = jnp.dot(kv_ref[:, :Dh], qt_ref[rs, cs], preferred_element_type=f32)
            m = jnp.max(s, axis=0, keepdims=True)
            p = jnp.exp2(s - m)
            lsum = jnp.sum(p, axis=0, keepdims=True)
            acc = jnp.dot(vt_ref[...], p.astype(bf16), preferred_element_type=f32)
            ot_ref[rs, cs] = (acc / lsum).astype(bf16)
            return 0

        jax.lax.fori_loop(0, NU, exact, 0)

    def tail(i, _):
        r = pl.multiple_of(i * TQ, TQ)
        xn = xn_ref[pl.ds(r, TQ), :]
        attn = jax.lax.dot_general(ot_ref[:, pl.ds(r, TQ)], wo_ref[...],
                                   (((0,), (0,)), ((), ())), preferred_element_type=f32)
        hmid = jax.lax.dot_general(xn, w1t_ref[...], nt, preferred_element_type=f32)
        hmid = (hmid * jax.nn.sigmoid(hmid)).astype(bf16)
        ffn = jnp.dot(hmid, w2_ref[...], preferred_element_type=f32)
        o_ref[pl.ds(r, TQ), :] = (x_ref[pl.ds(r, TQ), :].astype(f32) + attn + ffn).astype(o_ref.dtype)
        return 0

    jax.lax.fori_loop(0, NQ, tail, 0)


@jax.jit
def pallas_parallel_sum__grouped_kv_mqa__dense_activation_silu__prompt_kernel(
    A_x: jax.Array,
    A_wq: jax.Array,
    A_wk: jax.Array,
    A_wv: jax.Array,
    A_wo: jax.Array,
    B_x: jax.Array,
    B_w1: jax.Array,
    B_w2: jax.Array,
):
    del B_x
    B, S, D = A_x.shape
    assert B == 1
    Dh = D // _H
    NC = S // _CK
    x = A_x.reshape(S, D)
    bf16, f32 = jnp.bfloat16, jnp.float32

    out = pl.pallas_call(
        functools.partial(_kernel, S=S, D=D, Dh=Dh),
        out_shape=jax.ShapeDtypeStruct((S, D), A_x.dtype),
        scratch_shapes=[
            pltpu.VMEM((S, D), bf16),
            pltpu.VMEM((D, D), bf16),
            pltpu.VMEM((D, S), bf16),
            pltpu.VMEM((S, 2 * Dh), bf16),
            pltpu.VMEM((NC * _NMG * _GR, Dh), bf16),
            pltpu.VMEM((Dh, NC * _GR, 128), f32),
            pltpu.VMEM((Dh, S), bf16),
            pltpu.VMEM((_TQ // 128, Dh, S), bf16),
            pltpu.VMEM((_UN, Dh, 8, _TQ), f32),
            pltpu.VMEM((D, S), bf16),
            pltpu.VMEM((_H, S), f32),
        ],
        compiler_params=pltpu.CompilerParams(vmem_limit_bytes=100 * 1024 * 1024),
    )(x, A_wq, A_wk.T, A_wv.T, A_wo, B_w1.T, B_w2)
    return out.reshape(B, S, D)
```

```python
import functools
import math

import jax
import jax.numpy as jnp
import jax.experimental.pallas as pl
import jax.experimental.pallas.tpu as pltpu

_H = 32
_EPS = 1e-5
_TQ = 512
_CK = 128
_GR = 16
_NG = _CK // _GR
_NMG = _NG - 1
_POS = (0, 2, 4, 6)
_UN = 8
_OFF = 2

_L_MIN = 2.0 ** -80
_L_MAX = 2.0 ** 100
_V_MAX = 2.0 ** 20


def _order(pos):
    o = list(range(_NMG))
    o.insert(pos, _NMG)
    return o


def _kernel(x_hbm, wq_hbm, wkt_hbm, wvt_hbm, wo_hbm, w1t_hbm, w2_hbm, o_hbm,
            x_ref, wq_ref, wo_ref, w1t_ref, w2_ref, out_ref,
            xn_ref, wqt_ref, qt_ref, kvt_ref, kv_ref, km_ref, kb_ref, vtp_ref,
            qs_ref, ot_ref, l_ref, in_sems, out_sems, *, S, D, Dh):
    f32, bf16, u32 = jnp.float32, jnp.bfloat16, jnp.uint32
    H, TQ, CK, GR, NMG, UN = _H, _TQ, _CK, _GR, _NMG, _UN
    NQ, NC, J = S // TQ, S // CK, TQ // 128
    NU, CPT = NQ * H, TQ // CK
    qscale = (Dh ** -0.5) * math.log2(math.e)
    nt = (((1,), (1,)), ((), ()))

    def x_copy(i):
        return pltpu.make_async_copy(x_hbm.at[pl.ds(i * TQ, TQ), :], x_ref.at[pl.ds(i * TQ, TQ), :],
                                     in_sems.at[i])

    wq_copy = pltpu.make_async_copy(wq_hbm, wq_ref, in_sems.at[NQ])
    wk_copy = pltpu.make_async_copy(wkt_hbm, wqt_ref.at[pl.ds(D, Dh), :], in_sems.at[NQ + 1])
    wv_copy = pltpu.make_async_copy(wvt_hbm, wqt_ref.at[pl.ds(D + Dh, Dh), :], in_sems.at[NQ + 2])
    late_copies = [pltpu.make_async_copy(src, dst, in_sems.at[NQ + 3 + n])
                   for n, (src, dst) in enumerate([(wo_hbm, wo_ref), (w1t_hbm, w1t_ref), (w2_hbm, w2_ref)])]
    x_copy(0).start()
    wq_copy.start()
    wk_copy.start()
    wv_copy.start()

    def layernorm(i):
        x = x_ref[pl.ds(i * TQ, TQ), :].astype(f32)
        mu = jnp.mean(x, axis=-1, keepdims=True)
        xc = x - mu
        var = jnp.mean(xc * xc, axis=-1, keepdims=True)
        xn_ref[pl.ds(i * TQ, TQ), :] = (xc * jax.lax.rsqrt(var + _EPS)).astype(bf16)

    def project(i):
        xn = xn_ref[pl.ds(i * TQ, TQ), :]
        qkv = jax.lax.dot_general(wqt_ref[...], xn, nt, preferred_element_type=f32)
        qt_ref[:, pl.ds(i * TQ, TQ)] = (qkv[:D] * qscale).astype(bf16)
        kvt_ref[:, pl.ds(i * TQ, TQ)] = qkv[D:].astype(bf16)

    src_key = jax.lax.broadcasted_iota(jnp.int32, (CK, CK), 0)
    dst_key = jax.lax.broadcasted_iota(jnp.int32, (CK, CK), 1)
    perms = []
    for j in range(J):
        want = jnp.zeros((CK, CK), jnp.int32)
        for slot, g in enumerate(reversed(_order(_POS[j]))):
            want = jnp.where(dst_key // GR == slot, g * GR + dst_key % GR, want)
        perms.append((src_key == want).astype(bf16))

    def tables(i):
        cs = range(i * CPT, (i + 1) * CPT)
        kvt = kvt_ref[:, pl.ds(i * TQ, TQ)]
        vstack = jnp.concatenate([kvt[Dh:, n * CK:(n + 1) * CK] for n in range(CPT)], axis=0)
        for j in range(J):
            vp = jnp.dot(vstack, perms[j], preferred_element_type=f32).astype(bf16)
            for n, c in enumerate(cs):
                vtp_ref[j, :, pl.ds(c * CK, CK)] = pltpu.bitcast(vp[n * Dh:(n + 1) * Dh, :], u32)
        kpad = jnp.concatenate([kvt.astype(f32), jnp.zeros((128 - 2 * Dh, TQ), f32)], axis=0)
        knat = kpad.T
        kv_ref[pl.ds(i * TQ, TQ), :] = knat.astype(bf16)
        for n, c in enumerate(cs):
            km_ref[pl.ds(c * NMG * GR // 2, NMG * GR // 2), :] = pltpu.bitcast(
                knat[n * CK:n * CK + NMG * GR, :].astype(bf16), u32)
            kf = knat[n * CK + NMG * GR:(n + 1) * CK, :]
            for d in range(Dh):
                kb_ref[d, pl.ds(c * GR, GR), :] = jnp.broadcast_to(kf[:, d:d + 1], (GR, 128))

    x_copy(0).wait()
    for i in range(1, NQ):
        x_copy(i).start()
    layernorm(0)
    wq_copy.wait()
    wk_copy.wait()
    wv_copy.wait()
    wqt_ref[pl.ds(0, D), :] = wq_ref[...].T
    for i in range(NQ):
        if i + 1 < NQ:
            x_copy(i + 1).wait()
            layernorm(i + 1)
        else:
            for cp in late_copies:
                cp.start()
        project(i)
        if i > 0:
            tables(i - 1)
    tables(NQ - 1)
    vmax = jnp.max(jnp.abs(kvt_ref[pl.ds(Dh, Dh), :].astype(f32)))

    def unit_slices(u):
        h = u % H
        j = u // H
        return (pl.ds(pl.multiple_of(h * Dh, Dh), Dh), pl.ds(pl.multiple_of(j * TQ, TQ), TQ), h)

    def fast(i, _):
        sts, qts, srows = {}, {}, {}
        per_unit = NC * NMG
        total = UN * per_unit

        def start(t):
            rs, cs, _h = unit_slices(i * UN + t)
            qts[t] = qt_ref[rs, cs]
            qs_ref[t] = qts[t].astype(f32)
            sts[t] = dict(l=[jnp.zeros((8, 128), f32)] * J, acc=[jnp.zeros((Dh, 128), f32)] * J)

        def finish(t):
            rs, cs, h = unit_slices(i * UN + t)
            lsum = jnp.sum(jnp.concatenate(sts[t]['l'], axis=1), axis=0, keepdims=True)
            l_ref[pl.ds(h, 1), cs] = lsum
            ot_ref[rs, cs] = (jnp.concatenate(sts[t]['acc'], axis=1) / lsum).astype(bf16)

        def mxu_scores(a, b):
            while a < b:
                t = a // per_unit
                e = min(b, (t + 1) * per_unit)
                if t not in qts:
                    start(t)
                la, le = a - t * per_unit, e - t * per_unit
                kk = pltpu.bitcast(km_ref[pl.ds(la * GR // 2, (le - la) * GR // 2), :], bf16)[:, :Dh]
                ss = [jnp.dot(kk, qts[t][:, j * 128:(j + 1) * 128], preferred_element_type=f32)
                      for j in range(J)]
                for j in range(J):
                    for xg in range(la, le):
                        r = srows.setdefault((t, xg // NMG, j), [None] * (2 * _NG))
                        g, o = xg % NMG, (xg - la) * GR
                        r[2 * g] = ss[j][o:o + 8, :]
                        r[2 * g + 1] = ss[j][o + 8:o + 16, :]
                a = e

        def vpu_scores(t, c, j):
            acc = [None, None]
            for d in range(Dh):
                qb = jnp.broadcast_to(qs_ref[t, pl.ds(d, 1), pl.ds(j * 128, 128)], (8, 128))
                for half in range(2):
                    y = kb_ref[d, pl.ds(c * GR + 8 * half, 8), :] * qb
                    acc[half] = y if d == 0 else acc[half] + y
            return acc

        def pv(t, c, j, rows):
            st, order = sts[t], _order(_POS[j])
            ps = {}
            for g in order:
                ps[2 * g] = jnp.exp2(rows[2 * g])
                ps[2 * g + 1] = jnp.exp2(rows[2 * g + 1])
            lc = ps[0]
            for r in range(1, 2 * _NG):
                lc = lc + ps[r]
            st['l'][j] = st['l'][j] + lc
            grp = []
            for g in reversed(order):
                grp += [ps[2 * g], ps[2 * g + 1]]
            p = jnp.concatenate(grp, axis=0).astype(bf16)
            vv = pltpu.bitcast(vtp_ref[j, :, pl.ds(c * CK, CK)], bf16)
            st['acc'][j] = st['acc'][j] + jnp.dot(vv, p, preferred_element_type=f32)

        mxu_scores(0, NMG)
        done = NMG
        for t in range(UN):
            for c in range(NC):
                need = min(total, (t * NC + c + 2) * NMG + _OFF)
                mxu_scores(done, need)
                done = need
                for j in range(J):
                    r = srows.pop((t, c, j))
                    r[2 * NMG], r[2 * NMG + 1] = vpu_scores(t, c, j)
                    pv(t, c, j, r)
                if c == NC - 1:
                    finish(t)
        return 0

    jax.lax.fori_loop(0, NU // UN, fast, 0)

    lall = l_ref[...]
    l_ok = jnp.logical_and(lall >= _L_MIN, lall <= _L_MAX)
    n_bad = jnp.sum(jnp.where(l_ok, 0.0, 1.0))
    safe = jnp.logical_and(n_bad == 0.0, vmax <= _V_MAX)

    @pl.when(jnp.logical_not(safe))
    def _():
        def exact(u, _):
            rs, cs, _h = unit_slices(u)
            s = jnp.dot(kv_ref[:, :Dh], qt_ref[rs, cs], preferred_element_type=f32)
            m = jnp.max(s, axis=0, keepdims=True)
            p = jnp.exp2(s - m)
            lsum = jnp.sum(p, axis=0, keepdims=True)
            acc = jnp.dot(kvt_ref[pl.ds(Dh, Dh), :], p.astype(bf16), preferred_element_type=f32)
            ot_ref[rs, cs] = (acc / lsum).astype(bf16)
            return 0

        jax.lax.fori_loop(0, NU, exact, 0)

    for cp in late_copies:
        cp.wait()

    def out_copy(i):
        r = pl.multiple_of(i * TQ, TQ)
        return pltpu.make_async_copy(out_ref.at[pl.ds(r, TQ), :], o_hbm.at[pl.ds(r, TQ), :],
                                     out_sems.at[i])

    def tail(i, _):
        r = pl.multiple_of(i * TQ, TQ)
        xn = xn_ref[pl.ds(r, TQ), :]
        attn = jax.lax.dot_general(ot_ref[:, pl.ds(r, TQ)], wo_ref[...],
                                   (((0,), (0,)), ((), ())), preferred_element_type=f32)
        hmid = jax.lax.dot_general(xn, w1t_ref[...], nt, preferred_element_type=f32)
        hmid = (hmid * jax.nn.sigmoid(hmid)).astype(bf16)
        ffn = jnp.dot(hmid, w2_ref[...], preferred_element_type=f32)
        out_ref[pl.ds(r, TQ), :] = (x_ref[pl.ds(r, TQ), :].astype(f32) + attn + ffn).astype(out_ref.dtype)
        out_copy(i).start()
        return 0

    jax.lax.fori_loop(0, NQ, tail, 0)
    for i in range(NQ):
        out_copy(i).wait()


@jax.jit
def pallas_parallel_sum__grouped_kv_mqa__dense_activation_silu__prompt_kernel(
    A_x: jax.Array,
    A_wq: jax.Array,
    A_wk: jax.Array,
    A_wv: jax.Array,
    A_wo: jax.Array,
    B_x: jax.Array,
    B_w1: jax.Array,
    B_w2: jax.Array,
):
    del B_x
    B, S, D = A_x.shape
    assert B == 1
    F = B_w1.shape[1]
    Dh = D // _H
    NC, NQ = S // _CK, S // _TQ
    x = A_x.reshape(S, D)
    bf16, f32, u32 = jnp.bfloat16, jnp.float32, jnp.uint32
    hbm = pl.BlockSpec(memory_space=pl.ANY)

    out = pl.pallas_call(
        functools.partial(_kernel, S=S, D=D, Dh=Dh),
        out_shape=jax.ShapeDtypeStruct((S, D), A_x.dtype),
        in_specs=[hbm] * 7,
        out_specs=hbm,
        scratch_shapes=[
            pltpu.VMEM((S, D), bf16),
            pltpu.VMEM((D, D), bf16),
            pltpu.VMEM((D, D), bf16),
            pltpu.VMEM((F, D), bf16),
            pltpu.VMEM((F, D), bf16),
            pltpu.VMEM((S, D), A_x.dtype),
            pltpu.VMEM((S, D), bf16),
            pltpu.VMEM((D + 2 * Dh, D), bf16),
            pltpu.VMEM((D, S), bf16),
            pltpu.VMEM((2 * Dh, S), bf16),
            pltpu.VMEM((S, 128), bf16),
            pltpu.VMEM((NC * _NMG * _GR // 2, 128), u32),
            pltpu.VMEM((Dh, NC * _GR, 128), f32),
            pltpu.VMEM((_TQ // 128, Dh // 2, S), u32),
            pltpu.VMEM((_UN, Dh, _TQ), f32),
            pltpu.VMEM((D, S), bf16),
            pltpu.VMEM((_H, S), f32),
            pltpu.SemaphoreType.DMA((NQ + 6,)),
            pltpu.SemaphoreType.DMA((NQ,)),
        ],
        compiler_params=pltpu.CompilerParams(vmem_limit_bytes=100 * 1024 * 1024),
    )(x, A_wq, A_wk.T, A_wv.T, A_wo, B_w1.T, B_w2)
    return out.reshape(B, S, D)
```

```python
import functools
import math

import jax
import jax.numpy as jnp
import jax.experimental.pallas as pl
import jax.experimental.pallas.tpu as pltpu

_H = 32
_EPS = 1e-5
_TQ = 512
_J = _TQ // 128
_CK = 128
_NH = _CK // 8
_UN = 16

_POS = (0, 2, 4, 7)
_MIX = (12, 12, 10, 12)
_OFF = 3

_L_MIN = 2.0 ** -80
_L_MAX = 2.0 ** 100
_V_MAX = 2.0 ** 20


def _n_vpu(j, c):
    return 3 if c % _J == j else 2


def _slots(j, extra):
    m = list(range(_NH - 3)) if extra else list(range(_NH - 2))
    if extra:
        m.insert(_MIX[j] + 1, _NH - 3)
    o = [(m[2 * i], m[2 * i + 1]) for i in range(len(m) // 2)]
    o.insert(_POS[j], (_NH - 2, _NH - 1))
    return o


def _kernel(x_hbm, wq_hbm, wkt_hbm, wvt_hbm, wo_hbm, w1t_hbm, w2_hbm, o_hbm,
            x_ref, wq_ref, wo_ref, w1t_ref, w2_ref, out_ref,
            xn_ref, wqt_ref, qt_ref, kvt_ref, kf_ref, km_ref, km2_ref, kb_ref, vtp_ref,
            qs_ref, acc_ref, l_ref, zero_ref, in_sems, out_sems, *, S, D, Dh):
    f32, bf16, u32 = jnp.float32, jnp.bfloat16, jnp.uint32
    H, TQ, J, CK, NH, UN = _H, _TQ, _J, _CK, _NH, _UN
    NQ, NC = S // TQ, S // CK
    NU, CPT = NQ * H, TQ // CK
    qscale = (Dh ** -0.5) * math.log2(math.e)
    nt = (((1,), (1,)), ((), ()))

    stream = [[(c, x) for c in range(NC) for x in range(NH - _n_vpu(j, c))] for j in range(J)]
    first = [[sum(NH - _n_vpu(j, cc) for cc in range(c)) for c in range(NC + 1)] for j in range(J)]
    per = len(stream[0]) // 2

    def x_copy(i):
        return pltpu.make_async_copy(x_hbm.at[pl.ds(i * TQ, TQ), :], x_ref.at[pl.ds(i * TQ, TQ), :],
                                     in_sems.at[i])

    wq_copy = pltpu.make_async_copy(wq_hbm, wq_ref, in_sems.at[NQ])
    wk_copy = pltpu.make_async_copy(wkt_hbm, wqt_ref.at[pl.ds(D, Dh), :], in_sems.at[NQ + 1])
    wv_copy = pltpu.make_async_copy(wvt_hbm, wqt_ref.at[pl.ds(D + Dh, Dh), :], in_sems.at[NQ + 2])
    late_copies = [pltpu.make_async_copy(src, dst, in_sems.at[NQ + 3 + n])
                   for n, (src, dst) in enumerate([(wo_hbm, wo_ref), (w1t_hbm, w1t_ref), (w2_hbm, w2_ref)])]
    wq_copy.start()
    x_copy(0).start()
    wk_copy.start()
    wv_copy.start()

    def layernorm(i):
        x = x_ref[pl.ds(i * TQ, TQ), :].astype(f32)
        mu = jnp.mean(x, axis=-1, keepdims=True)
        xc = x - mu
        var = jnp.mean(xc * xc, axis=-1, keepdims=True)
        xn_ref[pl.ds(i * TQ, TQ), :] = (xc * jax.lax.rsqrt(var + _EPS)).astype(bf16)

    def project_a(i):
        xn = xn_ref[pl.ds(i * TQ, TQ), :]
        r = jax.lax.dot_general(wqt_ref[pl.ds(D // 2, D // 2 + 2 * Dh), :], xn, nt, preferred_element_type=f32)
        qt_ref[pl.ds(D // 2, D // 2), pl.ds(i * TQ, TQ)] = (r[:D // 2] * qscale).astype(bf16)
        kvt_ref[:, pl.ds(i * TQ, TQ)] = r[D // 2:].astype(bf16)

    def project_b(i):
        xn = xn_ref[pl.ds(i * TQ, TQ), :]
        r = jax.lax.dot_general(wqt_ref[pl.ds(0, D // 2), :], xn, nt, preferred_element_type=f32)
        qt_ref[pl.ds(0, D // 2), pl.ds(i * TQ, TQ)] = (r * qscale).astype(bf16)

    src_key = jax.lax.broadcasted_iota(jnp.int32, (CK, CK), 0)
    dst_key = jax.lax.broadcasted_iota(jnp.int32, (CK, CK), 1)
    dst_row = jax.lax.broadcasted_iota(jnp.int32, (1, CK), 1)

    def perm(j, extra):
        halves = [x for pair in reversed(_slots(j, extra)) for x in pair]
        want = jnp.zeros((1, CK), jnp.int32)
        for slot, x in enumerate(halves):
            want = jnp.where(dst_row // 8 == slot, x * 8 + dst_row % 8, want)
        return (src_key == want).astype(bf16)

    perms = [[perm(j, extra) for extra in (False, True)] for j in range(J)]

    def tables(i):
        kvt = kvt_ref[:, pl.ds(i * TQ, TQ)]
        vts = [kvt[Dh:, n * CK:(n + 1) * CK] for n in range(CPT)]
        for j in range(J):
            for extra in (False, True):
                ns = [n for n in range(CPT) if (_n_vpu(j, i * CPT + n) == 3) == extra]
                vp = jnp.dot(jnp.concatenate([vts[n] for n in ns], axis=0), perms[j][extra],
                             preferred_element_type=f32).astype(bf16)
                for r, n in enumerate(ns):
                    vtp_ref[j, :, pl.ds((i * CPT + n) * CK, CK)] = pltpu.bitcast(vp[r * Dh:(r + 1) * Dh, :], u32)
        kt = kvt[:Dh].astype(f32)
        knat = jnp.concatenate([kt, jnp.zeros((128 - Dh, TQ), f32)], axis=0).T
        kf_ref[pl.ds(i * TQ, TQ), :] = knat
        for n in range(CPT):
            kv = knat[(n + 1) * CK - 24:(n + 1) * CK, :]
            for d in range(Dh):
                kb_ref[d, pl.ds((i * CPT + n) * 24, 24), :] = jnp.broadcast_to(kv[:, d:d + 1], (24, 128))
        if i % 2 == 1:
            c0, c1 = (i - 1) * CPT, (i + 1) * CPT
            for j in range(J):
                rows = jnp.concatenate([kf_ref[pl.ds(c * CK, 8 * (NH - _n_vpu(j, c))), :]
                                        for c in range(c0, c1)], axis=0)
                km_ref[j, pl.ds(first[j][c0] * 4, (first[j][c1] - first[j][c0]) * 4), :] = pltpu.bitcast(
                    rows.astype(bf16), u32)
        if i == 0:
            ksh = jnp.concatenate([jnp.zeros((Dh, CK), f32), kt[:, :CK],
                                   jnp.zeros((128 - 2 * Dh, CK), f32)], axis=0).T
            km2_ref[...] = pltpu.bitcast(ksh.astype(bf16), u32)

    zero_ref[...] = jnp.zeros(zero_ref.shape, f32)
    wq_copy.wait()
    eye = (src_key == dst_key).astype(bf16)
    for a in reversed(range(D // CK)):
        wqt_ref[pl.ds(a * CK, CK), :] = jax.lax.dot_general(
            eye, wq_ref[:, pl.ds(a * CK, CK)], nt, preferred_element_type=f32).astype(bf16)
    x_copy(0).wait()
    wk_copy.wait()
    wv_copy.wait()
    for i in range(1, NQ):
        x_copy(i).start()
    for i in range(NQ):
        if i > 0:
            if i < NQ - 1:
                x_copy(i).wait()
            if i == NQ - 2:
                x_copy(i + 1).wait()
            project_b(i - 1)
            tables(i - 1)
        layernorm(i)
        project_a(i)
    project_b(NQ - 1)
    tables(NQ - 1)
    vmax = jnp.max(jnp.abs(kvt_ref[pl.ds(Dh, Dh), :].astype(f32)))

    def head_rows(h):
        return pl.ds(pl.multiple_of(h * Dh, Dh), Dh)

    def q_cols(j):
        return pl.ds(pl.multiple_of(j * TQ, TQ), TQ)

    def fast(i, _):
        sts, qts, qbs, prows = {}, {}, {}, {}
        h0, cs = (i * UN) % H, q_cols((i * UN) // H)

        def get_q(t):
            if t not in qts:
                qts[t] = qt_ref[head_rows(h0 + t), cs]
                qs_ref[t] = qts[t].astype(f32)
                sts[t] = dict(l=[None] * J, acc=[None] * J)
            return qts[t]

        def finish(t):
            l_ref[pl.ds(h0 + t, 1), cs] = jnp.sum(jnp.concatenate(sts[t]['l'], axis=1), axis=0, keepdims=True)
            acc_ref[head_rows(h0 + t), cs] = jnp.concatenate(sts[t]['acc'], axis=1)

        def mxu_probs(j, a, b):
            if a >= b:
                return
            t0, t1 = a // per, (b - 1) // per
            la = a - t0 * per
            if t0 == t1:
                kk = km_ref[j, pl.ds(la * 8, (b - a) * 8), :]
                kk, w = pltpu.bitcast(kk, bf16)[:, :Dh], get_q(t0)
            else:
                kk = jnp.concatenate([km_ref[j, pl.ds(la * 8, (per - la) * 8), :],
                                      km2_ref[pl.ds(0, (b - t1 * per) * 8), :]], axis=0)
                kk = pltpu.bitcast(kk, bf16)[:, :2 * Dh]
                w = jnp.concatenate([get_q(t0), get_q(t1)], axis=0)
            p = jnp.exp2(jnp.dot(kk, w[:, j * 128:(j + 1) * 128], preferred_element_type=f32))
            for x in range(2 * a, 2 * b):
                c, hx = stream[j][x % (2 * per)]
                o = (x - 2 * a) * 8
                prows.setdefault((x // (2 * per), c, j), [None] * NH)[hx] = p[o:o + 8, :]

        def vpu_probs(t, j, kb):
            acc = None
            for d in range(Dh):
                if (t, d, j) not in qbs:
                    qbs[(t, d, j)] = qs_ref[t, pl.ds(d, 1), pl.ds(j * 128, 128)]
                y = kb[d] * jnp.broadcast_to(qbs[(t, d, j)], kb[d].shape)
                acc = y if d == 0 else acc + y
            return jnp.exp2(acc)

        def pv(t, c, j, ps):
            st = sts[t]
            lc = jnp.sum(jnp.concatenate(ps, axis=0).reshape(NH, 8, 128), axis=0)
            st['l'][j] = lc if c == 0 else st['l'][j] + lc
            order = [x for pair in reversed(_slots(j, _n_vpu(j, c) == 3)) for x in pair]
            p = jnp.concatenate([ps[x] for x in order], axis=0).astype(bf16)
            vv = pltpu.bitcast(vtp_ref[j, :, pl.ds(c * CK, CK)], bf16)
            a = jnp.dot(vv, p, preferred_element_type=f32)
            st['acc'][j] = (zero_ref[...] if c == 0 else st['acc'][j]) + a

        def upto(j, gc):
            t, c = divmod(gc, NC)
            return t * per + (first[j][c] + 1) // 2

        done = [upto(j, 1) for j in range(J)]
        for j in range(J):
            mxu_probs(j, 0, done[j])
        for t in range(UN):
            for c in range(NC):
                for j in range(J):
                    need = min(UN * per, upto(j, t * NC + c + 2) + _OFF)
                    mxu_probs(j, done[j], need)
                    done[j] = need
                kb2 = kb_ref[:, pl.ds(c * 24 + 8, 16), :]
                kb2 = [kb2[d] for d in range(Dh)]
                for j in range(J):
                    ps = prows.pop((t, c, j))
                    p2 = vpu_probs(t, j, kb2)
                    ps[NH - 2], ps[NH - 1] = p2[:8], p2[8:]
                    if _n_vpu(j, c) == 3:
                        kb1 = kb_ref[:, pl.ds(c * 24, 8), :]
                        ps[NH - 3] = vpu_probs(t, j, [kb1[d] for d in range(Dh)])
                    pv(t, c, j, ps)
                if c == NC - 1:
                    finish(t)
        return 0

    for cp in late_copies:
        cp.start()
    jax.lax.fori_loop(0, NU // UN, fast, 0)

    lall = l_ref[...]
    l_ok = jnp.logical_and(lall >= _L_MIN, lall <= _L_MAX)
    n_bad = jnp.sum(jnp.where(l_ok, 0.0, 1.0))
    safe = jnp.logical_and(n_bad == 0.0, vmax <= _V_MAX)

    @pl.when(jnp.logical_not(safe))
    def _():
        def exact(u, _):
            h, cs = u % H, q_cols(u // H)
            s = jnp.dot(kf_ref[...].astype(bf16)[:, :Dh], qt_ref[head_rows(h), cs], preferred_element_type=f32)
            m = jnp.max(s, axis=0, keepdims=True)
            p = jnp.exp2(s - m)
            l_ref[pl.ds(h, 1), cs] = jnp.sum(p, axis=0, keepdims=True)
            acc_ref[head_rows(h), cs] = jnp.dot(kvt_ref[pl.ds(Dh, Dh), :], p.astype(bf16),
                                                preferred_element_type=f32)
            return 0

        jax.lax.fori_loop(0, NU, exact, 0)

    for cp in late_copies:
        cp.wait()

    def out_copy(i):
        return pltpu.make_async_copy(out_ref.at[q_cols(i), :], o_hbm.at[q_cols(i), :], out_sems.at[i])

    def tail(i, _):
        rs = q_cols(i)
        hmid = jax.lax.dot_general(xn_ref[rs, :], w1t_ref[...], nt, preferred_element_type=f32)
        hmid = (hmid * jax.nn.sigmoid(hmid)).astype(bf16)
        rinv = 1.0 / l_ref[:, rs]
        ot = (acc_ref[:, rs].reshape(H, Dh, TQ) * rinv[:, None, :]).reshape(D, TQ).astype(bf16)
        attn = jax.lax.dot_general(ot, wo_ref[...], (((0,), (0,)), ((), ())), preferred_element_type=f32)
        ffn = jnp.dot(hmid, w2_ref[...], preferred_element_type=f32)
        out_ref[rs, :] = (x_ref[rs, :].astype(f32) + attn + ffn).astype(out_ref.dtype)
        out_copy(i).start()
        return 0

    jax.lax.fori_loop(0, NQ, tail, 0)
    for i in range(NQ):
        out_copy(i).wait()


@jax.jit
def pallas_parallel_sum__grouped_kv_mqa__dense_activation_silu__prompt_kernel(
    A_x: jax.Array,
    A_wq: jax.Array,
    A_wk: jax.Array,
    A_wv: jax.Array,
    A_wo: jax.Array,
    B_x: jax.Array,
    B_w1: jax.Array,
    B_w2: jax.Array,
):
    del B_x
    B, S, D = A_x.shape
    assert B == 1
    F = B_w1.shape[1]
    Dh = D // _H
    NC, NQ = S // _CK, S // _TQ
    n_mxu = sum(_NH - _n_vpu(0, c) for c in range(NC))
    x = A_x.reshape(S, D)
    bf16, f32, u32 = jnp.bfloat16, jnp.float32, jnp.uint32
    hbm = pl.BlockSpec(memory_space=pl.ANY)

    out = pl.pallas_call(
        functools.partial(_kernel, S=S, D=D, Dh=Dh),
        out_shape=jax.ShapeDtypeStruct((S, D), A_x.dtype),
        in_specs=[hbm] * 7,
        out_specs=hbm,
        scratch_shapes=[
            pltpu.VMEM((S, D), bf16),
            pltpu.VMEM((D, D), bf16),
            pltpu.VMEM((D, D), bf16),
            pltpu.VMEM((F, D), bf16),
            pltpu.VMEM((F, D), bf16),
            pltpu.VMEM((S, D), A_x.dtype),
            pltpu.VMEM((S, D), bf16),
            pltpu.VMEM((D + 2 * Dh, D), bf16),
            pltpu.VMEM((D, S), bf16),
            pltpu.VMEM((2 * Dh, S), bf16),
            pltpu.VMEM((S, 128), f32),
            pltpu.VMEM((_J, n_mxu * 4, 128), u32),
            pltpu.VMEM((_CK // 2, 128), u32),
            pltpu.VMEM((Dh, NC * 24, 128), f32),
            pltpu.VMEM((_J, Dh // 2, S), u32),
            pltpu.VMEM((_UN, Dh, _TQ), f32),
            pltpu.VMEM((D, S), f32),
            pltpu.VMEM((_H, S), f32),
            pltpu.VMEM((Dh, 128), f32),
            pltpu.SemaphoreType.DMA((NQ + 6,)),
            pltpu.SemaphoreType.DMA((NQ,)),
        ],
        compiler_params=pltpu.CompilerParams(vmem_limit_bytes=100 * 1024 * 1024),
    )(x, A_wq, A_wk.T, A_wv.T, A_wo, B_w1.T, B_w2)
    return out.reshape(B, S, D)
```

```python
import functools
import math

import jax
import jax.numpy as jnp
import jax.experimental.pallas as pl
import jax.experimental.pallas.tpu as pltpu

_H = 32
_EPS = 1e-5
_TQ = 512
_J = _TQ // 128
_CK = 128
_NH = _CK // 8
_UN = 16

_EXTRA = ((0, 1), (2, 3))
_POS = (0, 5, 7, 14)
_XP = (13, 10, 11, 9)
_OFF = (2, 1, 1, 1)

_L_MIN = 2.0 ** -30
_L_MAX = 2.0 ** 100
_V_MAX = 2.0 ** 20


def _n_vpu(j, c):
    return 3 if j in _EXTRA[c % len(_EXTRA)] else 2


def _order(j, extra):
    o = list(range(_NH - 3 if extra else _NH - 2))
    if extra:
        o.insert(min(_XP[j], len(o)), _NH - 3)
    p = min(_POS[j], len(o))
    o[p:p] = [_NH - 2, _NH - 1]
    return o


def _kernel(x_hbm, wq_hbm, wkt_hbm, wvt_hbm, wo_hbm, w1t_hbm, w2_hbm, o_hbm,
            x_ref, wq_ref, wo_ref, w1t_ref, w2_ref, out_ref,
            xn_ref, wqt_ref, qt_ref, kvt_ref, kf_ref, km_ref, km2_ref, kb_ref, vtp_ref,
            qs_ref, acc_ref, l_ref, zero_ref, in_sems, out_sems, *, S, D, Dh):
    f32, bf16, u32 = jnp.float32, jnp.bfloat16, jnp.uint32
    H, TQ, J, CK, NH, UN = _H, _TQ, _J, _CK, _NH, _UN
    NQ, NC = S // TQ, S // CK
    NU, CPT = NQ * H, TQ // CK
    qscale = (Dh ** -0.5) * math.log2(math.e)
    nt = (((1,), (1,)), ((), ()))

    stream = [[(c, x) for c in range(NC) for x in range(NH - _n_vpu(j, c))] for j in range(J)]
    first = [[sum(NH - _n_vpu(j, cc) for cc in range(c)) for c in range(NC + 1)] for j in range(J)]
    per = len(stream[0]) // 2

    def x_copy(i):
        return pltpu.make_async_copy(x_hbm.at[pl.ds(i * TQ, TQ), :], x_ref.at[pl.ds(i * TQ, TQ), :],
                                     in_sems.at[i])

    wq_copy = pltpu.make_async_copy(wq_hbm, wq_ref, in_sems.at[NQ])
    wk_copy = pltpu.make_async_copy(wkt_hbm, wqt_ref.at[pl.ds(D, Dh), :], in_sems.at[NQ + 1])
    wv_copy = pltpu.make_async_copy(wvt_hbm, wqt_ref.at[pl.ds(D + Dh, Dh), :], in_sems.at[NQ + 2])
    late_copies = [pltpu.make_async_copy(src, dst, in_sems.at[NQ + 3 + n])
                   for n, (src, dst) in enumerate([(wo_hbm, wo_ref), (w1t_hbm, w1t_ref), (w2_hbm, w2_ref)])]
    wk_copy.start()
    wv_copy.start()
    wq_copy.start()
    x_copy(0).start()

    def layernorm(i):
        x = x_ref[pl.ds(i * TQ, TQ), :].astype(f32)
        mu = jnp.mean(x, axis=-1, keepdims=True)
        xc = x - mu
        var = jnp.mean(xc * xc, axis=-1, keepdims=True)
        xn_ref[pl.ds(i * TQ, TQ), :] = (xc * jax.lax.rsqrt(var + _EPS)).astype(bf16)

    def project_a(i):
        xn = xn_ref[pl.ds(i * TQ, TQ), :]
        r = jax.lax.dot_general(wqt_ref[pl.ds(D // 2, D // 2 + 2 * Dh), :], xn, nt, preferred_element_type=f32)
        qt_ref[pl.ds(D // 2, D // 2), pl.ds(i * TQ, TQ)] = (r[:D // 2] * qscale).astype(bf16)
        kvt_ref[:, pl.ds(i * TQ, TQ)] = r[D // 2:].astype(bf16)

    def project_b(i):
        xn = xn_ref[pl.ds(i * TQ, TQ), :]
        r = jax.lax.dot_general(wqt_ref[pl.ds(0, D // 2), :], xn, nt, preferred_element_type=f32)
        qt_ref[pl.ds(0, D // 2), pl.ds(i * TQ, TQ)] = (r * qscale).astype(bf16)

    src_key = jax.lax.broadcasted_iota(jnp.int32, (CK, CK), 0)
    dst_key = jax.lax.broadcasted_iota(jnp.int32, (CK, CK), 1)
    dst_row = jax.lax.broadcasted_iota(jnp.int32, (1, CK), 1)

    def perm(j, extra):
        halves = list(reversed(_order(j, extra)))
        want = jnp.zeros((1, CK), jnp.int32)
        for slot, x in enumerate(halves):
            want = jnp.where(dst_row // 8 == slot, x * 8 + dst_row % 8, want)
        return (src_key == want).astype(bf16)

    perms = [[perm(j, extra) for extra in (False, True)] for j in range(J)]

    def tables(i):
        kvt = kvt_ref[:, pl.ds(i * TQ, TQ)]
        vts = [kvt[Dh:, n * CK:(n + 1) * CK] for n in range(CPT)]
        for j in range(J):
            for extra in (False, True):
                ns = [n for n in range(CPT) if (_n_vpu(j, i * CPT + n) == 3) == extra]
                if not ns:
                    continue
                vp = jnp.dot(jnp.concatenate([vts[n] for n in ns], axis=0), perms[j][extra],
                             preferred_element_type=f32)
                for r, n in enumerate(ns):
                    vtp_ref[j, :, pl.ds((i * CPT + n) * CK, CK)] = vp[r * Dh:(r + 1) * Dh, :]
        kt = kvt[:Dh].astype(f32)
        knat = jnp.concatenate([kt, jnp.zeros((128 - Dh, TQ), f32)], axis=0).T
        kf_ref[pl.ds(i * TQ, TQ), :] = knat
        for n in range(CPT):
            kv = knat[(n + 1) * CK - 24:(n + 1) * CK, :]
            for d in range(Dh):
                kb_ref[d, pl.ds((i * CPT + n) * 24, 24), :] = jnp.broadcast_to(kv[:, d:d + 1], (24, 128))
        if i % 2 == 1:
            c0, c1 = (i - 1) * CPT, (i + 1) * CPT
            for j in range(J):
                rows = jnp.concatenate([kf_ref[pl.ds(c * CK, 8 * (NH - _n_vpu(j, c))), :]
                                        for c in range(c0, c1)], axis=0)
                km_ref[j, pl.ds(first[j][c0] * 4, (first[j][c1] - first[j][c0]) * 4), :] = pltpu.bitcast(
                    rows.astype(bf16), u32)
        if i == 0:
            ksh = jnp.concatenate([jnp.zeros((Dh, CK), f32), kt[:, :CK],
                                   jnp.zeros((128 - 2 * Dh, CK), f32)], axis=0).T
            km2_ref[...] = pltpu.bitcast(ksh.astype(bf16), u32)

    zero_ref[...] = jnp.zeros(zero_ref.shape, f32)
    wk_copy.wait()
    wv_copy.wait()
    wq_copy.wait()
    eye = (src_key == dst_key).astype(bf16)
    for a in reversed(range(D // CK)):
        wqt_ref[pl.ds(a * CK, CK), :] = jax.lax.dot_general(
            eye, wq_ref[:, pl.ds(a * CK, CK)], nt, preferred_element_type=f32).astype(bf16)
    x_copy(0).wait()
    for i in range(1, NQ):
        x_copy(i).start()
    for i in range(NQ):
        if i > 0:
            if i < NQ - 1:
                x_copy(i).wait()
            if i == NQ - 2:
                x_copy(i + 1).wait()
            project_b(i - 1)
            tables(i - 1)
        layernorm(i)
        project_a(i)
    project_b(NQ - 1)
    tables(NQ - 1)
    vmax = jnp.max(jnp.abs(kvt_ref[pl.ds(Dh, Dh), :].astype(f32)))

    def head_rows(h):
        return pl.ds(pl.multiple_of(h * Dh, Dh), Dh)

    def q_cols(j):
        return pl.ds(pl.multiple_of(j * TQ, TQ), TQ)

    def fast(i, _):
        sts, qts, qbs, kbs, prows = {}, {}, {}, {}, {}
        h0, cs = (i * UN) % H, q_cols((i * UN) // H)

        def get_q(t):
            if t not in qts:
                qts[t] = qt_ref[head_rows(h0 + t), cs]
                qs_ref[t] = qts[t].astype(f32)
                sts[t] = dict(l=[None] * J, acc=[None] * J)
            return qts[t]

        def finish(t):
            l_ref[pl.ds(h0 + t, 1), cs] = jnp.sum(jnp.concatenate(sts[t]['l'], axis=1), axis=0, keepdims=True)
            acc_ref[head_rows(h0 + t), cs] = jnp.concatenate(sts[t]['acc'], axis=1)

        def mxu_probs(j, a, b):
            if a >= b:
                return
            t0, t1 = a // per, (b - 1) // per
            la = a - t0 * per
            if t0 == t1:
                kk = km_ref[j, pl.ds(la * 8, (b - a) * 8), :]
                kk, w = pltpu.bitcast(kk, bf16)[:, :Dh], get_q(t0)
            else:
                kk = jnp.concatenate([km_ref[j, pl.ds(la * 8, (per - la) * 8), :],
                                      km2_ref[pl.ds(0, (b - t1 * per) * 8), :]], axis=0)
                kk = pltpu.bitcast(kk, bf16)[:, :2 * Dh]
                w = jnp.concatenate([get_q(t0), get_q(t1)], axis=0)
            p = jnp.exp2(jnp.dot(kk, w[:, j * 128:(j + 1) * 128], preferred_element_type=f32))
            x = 2 * a
            while x < 2 * b:
                t, lx = divmod(x, 2 * per)
                c = stream[j][lx][0]
                e = min(2 * b, t * 2 * per + first[j][c + 1])
                prows.setdefault((t, c, j), []).append(p[(x - 2 * a) * 8:(e - 2 * a) * 8, :])
                x = e

        def vpu_probs(t, j, row, n):
            if (row, n) not in kbs:
                kb = kb_ref[:, pl.ds(row, n), :]
                kbs[(row, n)] = [kb[d] for d in range(Dh)]
            acc = None
            for d in range(Dh):
                if (t, d, j, n) not in qbs:
                    qbs[(t, d, j, n)] = jnp.broadcast_to(qs_ref[t, pl.ds(d, 1), pl.ds(j * 128, 128)], (n, 128))
                y = kbs[(row, n)][d] * qbs[(t, d, j, n)]
                acc = y if d == 0 else acc + y
            return jnp.exp2(acc)

        def pv(t, c, j, pn):
            st = sts[t]
            lc = jnp.sum(pn.reshape(NH, 8, 128), axis=0)
            st['l'][j] = lc if c == 0 else st['l'][j] + lc
            p = jnp.concatenate([pn[x * 8:x * 8 + 8] for x in reversed(_order(j, _n_vpu(j, c) == 3))], axis=0)
            a = jnp.dot(vtp_ref[j, :, pl.ds(c * CK, CK)], p, preferred_element_type=f32)
            st['acc'][j] = (zero_ref[...] if c == 0 else st['acc'][j]) + a

        def upto(j, gc):
            t, c = divmod(gc, NC)
            return t * per + (first[j][c] + 1) // 2

        done = [upto(j, 1) for j in range(J)]
        for j in range(J):
            mxu_probs(j, 0, done[j])
        for t in range(UN):
            for c in range(NC):
                for j in range(J):
                    need = min(UN * per, upto(j, t * NC + c + 2) + _OFF[j])
                    mxu_probs(j, done[j], need)
                    done[j] = need
                for j in range(J):
                    ps = prows.pop((t, c, j))
                    p2 = vpu_probs(t, j, c * 24 + 8, 16)
                    if _n_vpu(j, c) == 3:
                        ps.append(vpu_probs(t, j, c * 24, 8))
                    pv(t, c, j, jnp.concatenate(ps + [p2], axis=0))
                if c == NC - 1:
                    finish(t)
        return 0

    for cp in late_copies:
        cp.start()
    jax.lax.fori_loop(0, NU // UN, fast, 0)

    lall = l_ref[...]
    l_ok = jnp.logical_and(lall >= _L_MIN, lall <= _L_MAX)
    n_bad = jnp.sum(jnp.where(l_ok, 0.0, 1.0))
    safe = jnp.logical_and(n_bad == 0.0, vmax <= _V_MAX)

    @pl.when(jnp.logical_not(safe))
    def _():
        def exact(u, _):
            h, cs = u % H, q_cols(u // H)
            s = jnp.dot(kf_ref[...].astype(bf16)[:, :Dh], qt_ref[head_rows(h), cs], preferred_element_type=f32)
            m = jnp.max(s, axis=0, keepdims=True)
            p = jnp.exp2(s - m)
            l_ref[pl.ds(h, 1), cs] = jnp.sum(p, axis=0, keepdims=True)
            acc_ref[head_rows(h), cs] = jnp.dot(kvt_ref[pl.ds(Dh, Dh), :], p.astype(bf16),
                                                preferred_element_type=f32)
            return 0

        jax.lax.fori_loop(0, NU, exact, 0)

    for cp in late_copies:
        cp.wait()

    def out_copy(i):
        return pltpu.make_async_copy(out_ref.at[q_cols(i), :], o_hbm.at[q_cols(i), :], out_sems.at[i])

    def tail(i, _):
        rs = q_cols(i)
        hmid = jax.lax.dot_general(xn_ref[rs, :], w1t_ref[...], nt, preferred_element_type=f32)
        hmid = (hmid * jax.nn.sigmoid(hmid)).astype(bf16)
        rinv = 1.0 / l_ref[:, rs]
        ot = (acc_ref[:, rs].reshape(H, Dh, TQ) * rinv[:, None, :]).reshape(D, TQ).astype(bf16)
        attn = jax.lax.dot_general(ot, wo_ref[...], (((0,), (0,)), ((), ())), preferred_element_type=f32)
        ffn = jnp.dot(hmid, w2_ref[...], preferred_element_type=f32)
        out_ref[rs, :] = (x_ref[rs, :].astype(f32) + attn + ffn).astype(out_ref.dtype)
        out_copy(i).start()
        return 0

    jax.lax.fori_loop(0, NQ, tail, 0)
    for i in range(NQ):
        out_copy(i).wait()


@jax.jit
def pallas_parallel_sum__grouped_kv_mqa__dense_activation_silu__prompt_kernel(
    A_x: jax.Array,
    A_wq: jax.Array,
    A_wk: jax.Array,
    A_wv: jax.Array,
    A_wo: jax.Array,
    B_x: jax.Array,
    B_w1: jax.Array,
    B_w2: jax.Array,
):
    del B_x
    B, S, D = A_x.shape
    assert B == 1
    F = B_w1.shape[1]
    Dh = D // _H
    NC, NQ = S // _CK, S // _TQ
    n_mxu = sum(_NH - _n_vpu(0, c) for c in range(NC))
    x = A_x.reshape(S, D)
    bf16, f32, u32 = jnp.bfloat16, jnp.float32, jnp.uint32
    hbm = pl.BlockSpec(memory_space=pl.ANY)

    out = pl.pallas_call(
        functools.partial(_kernel, S=S, D=D, Dh=Dh),
        out_shape=jax.ShapeDtypeStruct((S, D), A_x.dtype),
        in_specs=[hbm] * 7,
        out_specs=hbm,
        scratch_shapes=[
            pltpu.VMEM((S, D), bf16),
            pltpu.VMEM((D, D), bf16),
            pltpu.VMEM((D, D), bf16),
            pltpu.VMEM((F, D), bf16),
            pltpu.VMEM((F, D), bf16),
            pltpu.VMEM((S, D), A_x.dtype),
            pltpu.VMEM((S, D), bf16),
            pltpu.VMEM((D + 2 * Dh, D), bf16),
            pltpu.VMEM((D, S), bf16),
            pltpu.VMEM((2 * Dh, S), bf16),
            pltpu.VMEM((S, 128), f32),
            pltpu.VMEM((_J, n_mxu * 4, 128), u32),
            pltpu.VMEM((_CK // 2, 128), u32),
            pltpu.VMEM((Dh, NC * 24, 128), f32),
            pltpu.VMEM((_J, Dh, S), f32),
            pltpu.VMEM((_UN, Dh, _TQ), f32),
            pltpu.VMEM((D, S), f32),
            pltpu.VMEM((_H, S), f32),
            pltpu.VMEM((Dh, 128), f32),
            pltpu.SemaphoreType.DMA((NQ + 6,)),
            pltpu.SemaphoreType.DMA((NQ,)),
        ],
        compiler_params=pltpu.CompilerParams(vmem_limit_bytes=100 * 1024 * 1024),
    )(x, A_wq, A_wk.T, A_wv.T, A_wo, B_w1.T, B_w2)
    return out.reshape(B, S, D)
```

```python
import functools
import math

import jax
import jax.numpy as jnp
import jax.experimental.pallas as pl
import jax.experimental.pallas.tpu as pltpu

_H = 32
_EPS = 1e-5
_TQ = 512
_J = _TQ // 128
_CK = 128
_NH = _CK // 8
_UN = 16

_EXTRA = ((0, 1), (2, 3))
_POS = (0, 5, 7, 13)
_XP = (13, 11, 9, 9)
_OFF = (2, 1, 1, 1)

_L_MIN = 2.0 ** -30
_L_MAX = 2.0 ** 100
_V_MAX = 2.0 ** 20


def _n_vpu(j, c):
    return 3 if j in _EXTRA[c % len(_EXTRA)] else 2


def _order(j, extra):
    o = list(range(_NH - 3 if extra else _NH - 2))
    if extra:
        o.insert(min(_XP[j], len(o)), _NH - 3)
    p = min(_POS[j], len(o))
    o[p:p] = [_NH - 2, _NH - 1]
    return o


def _kernel(x_hbm, wq_hbm, wkt_hbm, wvt_hbm, wo_hbm, w1t_hbm, w2_hbm, o_hbm,
            x_ref, wq_ref, wo_ref, w1t_ref, w2_ref, out_ref,
            xn_ref, wqt_ref, qt_ref, kvt_ref, kf_ref, km_ref, km2_ref, kb_ref, vtp_ref,
            qs_ref, acc_ref, l_ref, zero_ref, in_sems, out_sems, *, S, D, Dh):
    f32, bf16, u32 = jnp.float32, jnp.bfloat16, jnp.uint32
    H, TQ, J, CK, NH, UN = _H, _TQ, _J, _CK, _NH, _UN
    NQ, NC = S // TQ, S // CK
    NU, CPT = NQ * H, TQ // CK
    qscale = (Dh ** -0.5) * math.log2(math.e)
    nt = (((1,), (1,)), ((), ()))

    stream = [[(c, x) for c in range(NC) for x in range(NH - _n_vpu(j, c))] for j in range(J)]
    first = [[sum(NH - _n_vpu(j, cc) for cc in range(c)) for c in range(NC + 1)] for j in range(J)]
    per = len(stream[0]) // 2

    def x_copy(i):
        return pltpu.make_async_copy(x_hbm.at[pl.ds(i * TQ, TQ), :], x_ref.at[pl.ds(i * TQ, TQ), :],
                                     in_sems.at[i])

    wq_copy = pltpu.make_async_copy(wq_hbm, wq_ref, in_sems.at[NQ])
    wk_copy = pltpu.make_async_copy(wkt_hbm, wqt_ref.at[pl.ds(D, Dh), :], in_sems.at[NQ + 1])
    wv_copy = pltpu.make_async_copy(wvt_hbm, wqt_ref.at[pl.ds(D + Dh, Dh), :], in_sems.at[NQ + 2])
    late_copies = [pltpu.make_async_copy(src, dst, in_sems.at[NQ + 3 + n])
                   for n, (src, dst) in enumerate([(wo_hbm, wo_ref), (w1t_hbm, w1t_ref), (w2_hbm, w2_ref)])]
    wk_copy.start()
    wv_copy.start()
    wq_copy.start()
    x_copy(0).start()

    def layernorm(i):
        x = x_ref[pl.ds(i * TQ, TQ), :].astype(f32)
        mu = jnp.mean(x, axis=-1, keepdims=True)
        xc = x - mu
        var = jnp.mean(xc * xc, axis=-1, keepdims=True)
        xn_ref[pl.ds(i * TQ, TQ), :] = (xc * jax.lax.rsqrt(var + _EPS)).astype(bf16)

    def project_a(i):
        xn = xn_ref[pl.ds(i * TQ, TQ), :]
        r = jax.lax.dot_general(wqt_ref[pl.ds(D // 2, D // 2 + 2 * Dh), :], xn, nt, preferred_element_type=f32)
        qt_ref[pl.ds(D // 2, D // 2), pl.ds(i * TQ, TQ)] = (r[:D // 2] * qscale).astype(bf16)
        kvt_ref[:, pl.ds(i * TQ, TQ)] = r[D // 2:].astype(bf16)

    def project_b(i):
        xn = xn_ref[pl.ds(i * TQ, TQ), :]
        r = jax.lax.dot_general(wqt_ref[pl.ds(0, D // 2), :], xn, nt, preferred_element_type=f32)
        qt_ref[pl.ds(0, D // 2), pl.ds(i * TQ, TQ)] = (r * qscale).astype(bf16)

    src_key = jax.lax.broadcasted_iota(jnp.int32, (CK, CK), 0)
    dst_key = jax.lax.broadcasted_iota(jnp.int32, (CK, CK), 1)
    dst_row = jax.lax.broadcasted_iota(jnp.int32, (1, CK), 1)

    def perm(j, extra):
        halves = list(reversed(_order(j, extra)))
        want = jnp.zeros((1, CK), jnp.int32)
        for slot, x in enumerate(halves):
            want = jnp.where(dst_row // 8 == slot, x * 8 + dst_row % 8, want)
        return (src_key == want).astype(bf16)

    perms = [[perm(j, extra) for extra in (False, True)] for j in range(J)]

    def tables(i):
        kvt = kvt_ref[:, pl.ds(i * TQ, TQ)]
        vts = [kvt[Dh:, n * CK:(n + 1) * CK] for n in range(CPT)]
        for j in range(J):
            for extra in (False, True):
                ns = [n for n in range(CPT) if (_n_vpu(j, i * CPT + n) == 3) == extra]
                if not ns:
                    continue
                vp = jnp.dot(jnp.concatenate([vts[n] for n in ns], axis=0), perms[j][extra],
                             preferred_element_type=f32)
                for r, n in enumerate(ns):
                    vtp_ref[j, :, pl.ds((i * CPT + n) * CK, CK)] = vp[r * Dh:(r + 1) * Dh, :]
        kt = kvt[:Dh].astype(f32)
        knat = jnp.concatenate([kt, jnp.zeros((128 - Dh, TQ), f32)], axis=0).T
        kf_ref[pl.ds(i * TQ, TQ), :] = knat
        for n in range(CPT):
            kv = knat[(n + 1) * CK - 24:(n + 1) * CK, :]
            for d in range(Dh):
                kb_ref[d, pl.ds((i * CPT + n) * 24, 24), :] = jnp.broadcast_to(kv[:, d:d + 1], (24, 128))
        if i % 2 == 1:
            c0, c1 = (i - 1) * CPT, (i + 1) * CPT
            for j in range(J):
                rows = jnp.concatenate([kf_ref[pl.ds(c * CK, 8 * (NH - _n_vpu(j, c))), :]
                                        for c in range(c0, c1)], axis=0)
                km_ref[j, pl.ds(first[j][c0] * 4, (first[j][c1] - first[j][c0]) * 4), :] = pltpu.bitcast(
                    rows.astype(bf16), u32)
        if i == 0:
            ksh = jnp.concatenate([jnp.zeros((Dh, CK), f32), kt[:, :CK],
                                   jnp.zeros((128 - 2 * Dh, CK), f32)], axis=0).T
            km2_ref[...] = pltpu.bitcast(ksh.astype(bf16), u32)

    zero_ref[...] = jnp.zeros(zero_ref.shape, f32)
    wk_copy.wait()
    wv_copy.wait()
    wq_copy.wait()
    eye = (src_key == dst_key).astype(bf16)
    for a in reversed(range(D // CK)):
        wqt_ref[pl.ds(a * CK, CK), :] = jax.lax.dot_general(
            eye, wq_ref[:, pl.ds(a * CK, CK)], nt, preferred_element_type=f32).astype(bf16)
    x_copy(0).wait()
    for i in range(1, NQ):
        x_copy(i).start()
    for i in range(NQ):
        if i > 0:
            if i < NQ - 1:
                x_copy(i).wait()
            if i == NQ - 2:
                x_copy(i + 1).wait()
            project_b(i - 1)
            tables(i - 1)
        layernorm(i)
        project_a(i)
    project_b(NQ - 1)
    tables(NQ - 1)
    vmax = jnp.max(jnp.abs(kvt_ref[pl.ds(Dh, Dh), :].astype(f32)))

    def head_rows(h):
        return pl.ds(pl.multiple_of(h * Dh, Dh), Dh)

    def q_cols(j):
        return pl.ds(pl.multiple_of(j * TQ, TQ), TQ)

    def fast(i, _):
        sts, qts, qbs, kbs, prows = {}, {}, {}, {}, {}
        h0, cs = (i * UN) % H, q_cols((i * UN) // H)

        def get_q(t):
            if t not in qts:
                qts[t] = qt_ref[head_rows(h0 + t), cs]
                qs_ref[t] = qts[t].astype(f32)
                sts[t] = dict(l=[None] * J, acc=[None] * J)
            return qts[t]

        def finish(t):
            l_ref[pl.ds(h0 + t, 1), cs] = jnp.sum(jnp.concatenate(sts[t]['l'], axis=1), axis=0, keepdims=True)
            acc_ref[head_rows(h0 + t), cs] = jnp.concatenate(sts[t]['acc'], axis=1)

        def mxu_probs(j, a, b):
            if a >= b:
                return
            t0, t1 = a // per, (b - 1) // per
            la = a - t0 * per
            if t0 == t1:
                kk = km_ref[j, pl.ds(la * 8, (b - a) * 8), :]
                kk, w = pltpu.bitcast(kk, bf16)[:, :Dh], get_q(t0)
            else:
                kk = jnp.concatenate([km_ref[j, pl.ds(la * 8, (per - la) * 8), :],
                                      km2_ref[pl.ds(0, (b - t1 * per) * 8), :]], axis=0)
                kk = pltpu.bitcast(kk, bf16)[:, :2 * Dh]
                w = jnp.concatenate([get_q(t0), get_q(t1)], axis=0)
            p = jnp.exp2(jnp.dot(kk, w[:, j * 128:(j + 1) * 128], preferred_element_type=f32))
            x = 2 * a
            while x < 2 * b:
                t, lx = divmod(x, 2 * per)
                c = stream[j][lx][0]
                e = min(2 * b, t * 2 * per + first[j][c + 1])
                prows.setdefault((t, c, j), []).append(p[(x - 2 * a) * 8:(e - 2 * a) * 8, :])
                x = e

        def vpu_probs(t, js, row, n):
            if (row, n) not in kbs:
                kb = kb_ref[:, pl.ds(row, n), :]
                kb = jnp.concatenate([kb] * len(js), axis=2)
                kbs[(row, n)] = [kb[d] for d in range(Dh)]
            acc = None
            for d in range(Dh):
                if (t, d, js) not in qbs:
                    qbs[(t, d, js)] = jnp.concatenate([
                        jnp.broadcast_to(qs_ref[t, pl.ds(d, 1), pl.ds(j * 128, 128)], (n, 128)) for j in js], axis=1)
                y = kbs[(row, n)][d] * qbs[(t, d, js)]
                acc = y if d == 0 else acc + y
            p = jnp.exp2(acc)
            return {j: p[:, k * 128:(k + 1) * 128] for k, j in enumerate(js)}

        def pv(t, c, j, pn):
            st = sts[t]
            lc = jnp.sum(pn.reshape(NH, 8, 128), axis=0)
            st['l'][j] = lc if c == 0 else st['l'][j] + lc
            p = jnp.concatenate([pn[x * 8:x * 8 + 8] for x in reversed(_order(j, _n_vpu(j, c) == 3))], axis=0)
            a = jnp.dot(vtp_ref[j, :, pl.ds(c * CK, CK)], p, preferred_element_type=f32)
            st['acc'][j] = (zero_ref[...] if c == 0 else st['acc'][j]) + a

        def upto(j, gc):
            t, c = divmod(gc, NC)
            return t * per + (first[j][c] + 1) // 2

        done = [upto(j, 1) for j in range(J)]
        for j in range(J):
            mxu_probs(j, 0, done[j])
        for t in range(UN):
            for c in range(NC):
                for j in range(J):
                    need = min(UN * per, upto(j, t * NC + c + 2) + _OFF[j])
                    mxu_probs(j, done[j], need)
                    done[j] = need
                p2 = vpu_probs(t, tuple(range(J)), c * 24 + 8, 16)
                p1 = vpu_probs(t, _EXTRA[c % len(_EXTRA)], c * 24, 8)
                for j in range(J):
                    ps = prows.pop((t, c, j)) + ([p1[j]] if j in p1 else []) + [p2[j]]
                    pv(t, c, j, jnp.concatenate(ps, axis=0))
                if c == NC - 1:
                    finish(t)
        return 0

    for cp in late_copies:
        cp.start()
    jax.lax.fori_loop(0, NU // UN, fast, 0)

    lall = l_ref[...]
    l_ok = jnp.logical_and(lall >= _L_MIN, lall <= _L_MAX)
    n_bad = jnp.sum(jnp.where(l_ok, 0.0, 1.0))
    safe = jnp.logical_and(n_bad == 0.0, vmax <= _V_MAX)

    @pl.when(jnp.logical_not(safe))
    def _():
        def exact(u, _):
            h, cs = u % H, q_cols(u // H)
            s = jnp.dot(kf_ref[...].astype(bf16)[:, :Dh], qt_ref[head_rows(h), cs], preferred_element_type=f32)
            m = jnp.max(s, axis=0, keepdims=True)
            p = jnp.exp2(s - m)
            l_ref[pl.ds(h, 1), cs] = jnp.sum(p, axis=0, keepdims=True)
            acc_ref[head_rows(h), cs] = jnp.dot(kvt_ref[pl.ds(Dh, Dh), :], p.astype(bf16),
                                                preferred_element_type=f32)
            return 0

        jax.lax.fori_loop(0, NU, exact, 0)

    for cp in late_copies:
        cp.wait()

    def out_copy(i):
        return pltpu.make_async_copy(out_ref.at[q_cols(i), :], o_hbm.at[q_cols(i), :], out_sems.at[i])

    def tail(i, _):
        rs = q_cols(i)
        hmid = jax.lax.dot_general(xn_ref[rs, :], w1t_ref[...], nt, preferred_element_type=f32)
        hmid = (hmid * jax.nn.sigmoid(hmid)).astype(bf16)
        rinv = 1.0 / l_ref[:, rs]
        ot = (acc_ref[:, rs].reshape(H, Dh, TQ) * rinv[:, None, :]).reshape(D, TQ).astype(bf16)
        attn = jax.lax.dot_general(ot, wo_ref[...], (((0,), (0,)), ((), ())), preferred_element_type=f32)
        ffn = jnp.dot(hmid, w2_ref[...], preferred_element_type=f32)
        out_ref[rs, :] = (x_ref[rs, :].astype(f32) + attn + ffn).astype(out_ref.dtype)
        out_copy(i).start()
        return 0

    jax.lax.fori_loop(0, NQ, tail, 0)
    for i in range(NQ):
        out_copy(i).wait()


@jax.jit
def pallas_parallel_sum__grouped_kv_mqa__dense_activation_silu__prompt_kernel(
    A_x: jax.Array,
    A_wq: jax.Array,
    A_wk: jax.Array,
    A_wv: jax.Array,
    A_wo: jax.Array,
    B_x: jax.Array,
    B_w1: jax.Array,
    B_w2: jax.Array,
):
    del B_x
    B, S, D = A_x.shape
    assert B == 1
    F = B_w1.shape[1]
    Dh = D // _H
    NC, NQ = S // _CK, S // _TQ
    n_mxu = sum(_NH - _n_vpu(0, c) for c in range(NC))
    x = A_x.reshape(S, D)
    bf16, f32, u32 = jnp.bfloat16, jnp.float32, jnp.uint32
    hbm = pl.BlockSpec(memory_space=pl.ANY)

    out = pl.pallas_call(
        functools.partial(_kernel, S=S, D=D, Dh=Dh),
        out_shape=jax.ShapeDtypeStruct((S, D), A_x.dtype),
        in_specs=[hbm] * 7,
        out_specs=hbm,
        scratch_shapes=[
            pltpu.VMEM((S, D), bf16),
            pltpu.VMEM((D, D), bf16),
            pltpu.VMEM((D, D), bf16),
            pltpu.VMEM((F, D), bf16),
            pltpu.VMEM((F, D), bf16),
            pltpu.VMEM((S, D), A_x.dtype),
            pltpu.VMEM((S, D), bf16),
            pltpu.VMEM((D + 2 * Dh, D), bf16),
            pltpu.VMEM((D, S), bf16),
            pltpu.VMEM((2 * Dh, S), bf16),
            pltpu.VMEM((S, 128), f32),
            pltpu.VMEM((_J, n_mxu * 4, 128), u32),
            pltpu.VMEM((_CK // 2, 128), u32),
            pltpu.VMEM((Dh, NC * 24, 128), f32),
            pltpu.VMEM((_J, Dh, S), f32),
            pltpu.VMEM((_UN, Dh, _TQ), f32),
            pltpu.VMEM((D, S), f32),
            pltpu.VMEM((_H, S), f32),
            pltpu.VMEM((Dh, 128), f32),
            pltpu.SemaphoreType.DMA((NQ + 6,)),
            pltpu.SemaphoreType.DMA((NQ,)),
        ],
        compiler_params=pltpu.CompilerParams(vmem_limit_bytes=100 * 1024 * 1024),
    )(x, A_wq, A_wk.T, A_wv.T, A_wo, B_w1.T, B_w2)
    return out.reshape(B, S, D)
```

```python
import functools
import math

import jax
import jax.numpy as jnp
import jax.experimental.pallas as pl
import jax.experimental.pallas.tpu as pltpu

_H = 32
_EPS = 1e-5
_TQ = 512
_J = _TQ // 128
_CK = 128
_NH = _CK // 8
_UN = 16

_EXTRA = ((0, 1), (2, 3))
_POS = (0, 5, 7, 13)
_XP = (13, 11, 9, 9)
_OFF = (2, 1, 1, 1)

_L_MIN = 2.0 ** -30
_L_MAX = 2.0 ** 100
_V_MAX = 2.0 ** 20


def _n_vpu(j, c):
    return 3 if j in _EXTRA[c % len(_EXTRA)] else 2


def _order(j, extra):
    o = list(range(_NH - 3 if extra else _NH - 2))
    if extra:
        o.insert(min(_XP[j], len(o)), _NH - 3)
    p = min(_POS[j], len(o))
    o[p:p] = [_NH - 2, _NH - 1]
    return o


def _kernel(x_hbm, wq_hbm, wkt_hbm, wvt_hbm, wo_hbm, w1t_hbm, w2_hbm, o_hbm,
            x_ref, wq_ref, wo_ref, w1t_ref, w2_ref, out_ref,
            xn_ref, wqt_ref, qt_ref, kvt_ref, kf_ref, km_ref, km2_ref, kb_ref, vtp_ref,
            qs_ref, acc_ref, l_ref, zero_ref, in_sems, out_sems, *, S, D, Dh):
    f32, bf16, u32 = jnp.float32, jnp.bfloat16, jnp.uint32
    H, TQ, J, CK, NH, UN = _H, _TQ, _J, _CK, _NH, _UN
    NQ, NC = S // TQ, S // CK
    NU, CPT = NQ * H, TQ // CK
    qscale = (Dh ** -0.5) * math.log2(math.e)
    nt = (((1,), (1,)), ((), ()))

    stream = [[(c, x) for c in range(NC) for x in range(NH - _n_vpu(j, c))] for j in range(J)]
    first = [[sum(NH - _n_vpu(j, cc) for cc in range(c)) for c in range(NC + 1)] for j in range(J)]
    per = len(stream[0]) // 2

    def x_copy(i):
        return pltpu.make_async_copy(x_hbm.at[pl.ds(i * TQ, TQ), :], x_ref.at[pl.ds(i * TQ, TQ), :],
                                     in_sems.at[i])

    wq_copy = pltpu.make_async_copy(wq_hbm, wq_ref, in_sems.at[NQ])
    wk_copy = pltpu.make_async_copy(wkt_hbm, wqt_ref.at[pl.ds(D, Dh), :], in_sems.at[NQ + 1])
    wv_copy = pltpu.make_async_copy(wvt_hbm, wqt_ref.at[pl.ds(D + Dh, Dh), :], in_sems.at[NQ + 2])
    late_copies = [pltpu.make_async_copy(src, dst, in_sems.at[NQ + 3 + n])
                   for n, (src, dst) in enumerate([(wo_hbm, wo_ref), (w1t_hbm, w1t_ref), (w2_hbm, w2_ref)])]
    wk_copy.start()
    wv_copy.start()
    wq_copy.start()
    x_copy(0).start()

    def layernorm(i):
        x = x_ref[pl.ds(i * TQ, TQ), :].astype(f32)
        mu = jnp.mean(x, axis=-1, keepdims=True)
        xc = x - mu
        var = jnp.mean(xc * xc, axis=-1, keepdims=True)
        xn_ref[pl.ds(i * TQ, TQ), :] = (xc * jax.lax.rsqrt(var + _EPS)).astype(bf16)

    def project_a(i):
        xn = xn_ref[pl.ds(i * TQ, TQ), :]
        r = jax.lax.dot_general(wqt_ref[pl.ds(D // 2, D // 2 + 2 * Dh), :], xn, nt, preferred_element_type=f32)
        qt_ref[pl.ds(D // 2, D // 2), pl.ds(i * TQ, TQ)] = (r[:D // 2] * qscale).astype(bf16)
        kvt_ref[:, pl.ds(i * TQ, TQ)] = r[D // 2:].astype(bf16)

    def project_b(i):
        xn = xn_ref[pl.ds(i * TQ, TQ), :]
        r = jax.lax.dot_general(wqt_ref[pl.ds(0, D // 2), :], xn, nt, preferred_element_type=f32)
        qt_ref[pl.ds(0, D // 2), pl.ds(i * TQ, TQ)] = (r * qscale).astype(bf16)

    src_key = jax.lax.broadcasted_iota(jnp.int32, (CK, CK), 0)
    dst_key = jax.lax.broadcasted_iota(jnp.int32, (CK, CK), 1)
    dst_row = jax.lax.broadcasted_iota(jnp.int32, (1, CK), 1)

    def perm(j, extra):
        halves = list(reversed(_order(j, extra)))
        want = jnp.zeros((1, CK), jnp.int32)
        for slot, x in enumerate(halves):
            want = jnp.where(dst_row // 8 == slot, x * 8 + dst_row % 8, want)
        return (src_key == want).astype(bf16)

    perms = [[perm(j, extra) for extra in (False, True)] for j in range(J)]

    def tables(i):
        kvt = kvt_ref[:, pl.ds(i * TQ, TQ)]
        vts = [kvt[Dh:, n * CK:(n + 1) * CK] for n in range(CPT)]
        for j in range(J):
            for extra in (False, True):
                ns = [n for n in range(CPT) if (_n_vpu(j, i * CPT + n) == 3) == extra]
                if not ns:
                    continue
                vp = jnp.dot(jnp.concatenate([vts[n] for n in ns], axis=0), perms[j][extra],
                             preferred_element_type=f32)
                for r, n in enumerate(ns):
                    vtp_ref[j, :, pl.ds((i * CPT + n) * CK, CK)] = vp[r * Dh:(r + 1) * Dh, :]
        kt = kvt[:Dh].astype(f32)
        knat = jnp.concatenate([kt, jnp.zeros((128 - Dh, TQ), f32)], axis=0).T
        kf_ref[pl.ds(i * TQ, TQ), :] = knat
        for n in range(CPT):
            kv = knat[(n + 1) * CK - 24:(n + 1) * CK, :]
            for d in range(Dh):
                kb_ref[d, pl.ds((i * CPT + n) * 24, 24), :] = jnp.broadcast_to(kv[:, d:d + 1], (24, 128))
        c0, c1 = i * CPT, (i + 1) * CPT
        for g, js in enumerate(_EXTRA):
            j = js[0]
            rows = jnp.concatenate([knat[n * CK:n * CK + 8 * (NH - _n_vpu(j, c0 + n)), :]
                                    for n in range(CPT)], axis=0)
            km_ref[g, pl.ds(first[j][c0] * 4, (first[j][c1] - first[j][c0]) * 4), :] = pltpu.bitcast(
                rows.astype(bf16), u32)
        if i == 0:
            ksh = jnp.concatenate([jnp.zeros((Dh, CK), f32), kt[:, :CK],
                                   jnp.zeros((128 - 2 * Dh, CK), f32)], axis=0).T
            km2_ref[...] = pltpu.bitcast(ksh.astype(bf16), u32)

    zero_ref[...] = jnp.zeros(zero_ref.shape, f32)
    wk_copy.wait()
    wv_copy.wait()
    wq_copy.wait()
    eye = (src_key == dst_key).astype(bf16)
    for a in reversed(range(D // CK)):
        wqt_ref[pl.ds(a * CK, CK), :] = jax.lax.dot_general(
            eye, wq_ref[:, pl.ds(a * CK, CK)], nt, preferred_element_type=f32).astype(bf16)
    x_copy(0).wait()
    for i in range(1, NQ):
        x_copy(i).start()
    for i in range(NQ):
        if i > 0:
            if i < NQ - 1:
                x_copy(i).wait()
            if i == NQ - 2:
                x_copy(i + 1).wait()
            project_b(i - 1)
            tables(i - 1)
        layernorm(i)
        project_a(i)
    project_b(NQ - 1)
    tables(NQ - 1)
    vmax = jnp.max(jnp.abs(kvt_ref[pl.ds(Dh, Dh), :].astype(f32)))

    def head_rows(h):
        return pl.ds(pl.multiple_of(h * Dh, Dh), Dh)

    def q_cols(j):
        return pl.ds(pl.multiple_of(j * TQ, TQ), TQ)

    def fast(i, _):
        sts, qts, qbs, kbs, prows = {}, {}, {}, {}, {}
        h0, cs = (i * UN) % H, q_cols((i * UN) // H)

        def get_q(t):
            if t not in qts:
                qts[t] = qt_ref[head_rows(h0 + t), cs]
                qs_ref[t] = qts[t].astype(f32)
                sts[t] = dict(l=[None] * J, acc=[None] * J)
            return qts[t]

        def finish(t):
            l_ref[pl.ds(h0 + t, 1), cs] = jnp.sum(jnp.concatenate(sts[t]['l'], axis=1), axis=0, keepdims=True)
            acc_ref[head_rows(h0 + t), cs] = jnp.concatenate(sts[t]['acc'], axis=1)

        def mxu_probs(j, a, b):
            if a >= b:
                return
            t0, t1 = a // per, (b - 1) // per
            la = a - t0 * per
            g = [j in js for js in _EXTRA].index(True)
            if t0 == t1:
                kk = km_ref[g, pl.ds(la * 8, (b - a) * 8), :]
                kk, w = pltpu.bitcast(kk, bf16)[:, :Dh], get_q(t0)
            else:
                kk = jnp.concatenate([km_ref[g, pl.ds(la * 8, (per - la) * 8), :],
                                      km2_ref[pl.ds(0, (b - t1 * per) * 8), :]], axis=0)
                kk = pltpu.bitcast(kk, bf16)[:, :2 * Dh]
                w = jnp.concatenate([get_q(t0), get_q(t1)], axis=0)
            p = jnp.exp2(jnp.dot(kk, w[:, j * 128:(j + 1) * 128], preferred_element_type=f32))
            x = 2 * a
            while x < 2 * b:
                t, lx = divmod(x, 2 * per)
                c = stream[j][lx][0]
                e = min(2 * b, t * 2 * per + first[j][c + 1])
                prows.setdefault((t, c, j), []).append(p[(x - 2 * a) * 8:(e - 2 * a) * 8, :])
                x = e

        def vpu_probs(t, js, row, n):
            if (row, n) not in kbs:
                kb = kb_ref[:, pl.ds(row, n), :]
                kb = jnp.concatenate([kb] * len(js), axis=2)
                kbs[(row, n)] = [kb[d] for d in range(Dh)]
            acc = None
            for d in range(Dh):
                if (t, d, js) not in qbs:
                    qbs[(t, d, js)] = jnp.concatenate([
                        jnp.broadcast_to(qs_ref[t, pl.ds(d, 1), pl.ds(j * 128, 128)], (n, 128)) for j in js], axis=1)
                y = kbs[(row, n)][d] * qbs[(t, d, js)]
                acc = y if d == 0 else acc + y
            p = jnp.exp2(acc)
            return {j: p[:, k * 128:(k + 1) * 128] for k, j in enumerate(js)}

        def pv(t, c, j, pn):
            st = sts[t]
            lc = jnp.sum(pn.reshape(NH, 8, 128), axis=0)
            st['l'][j] = lc if c == 0 else st['l'][j] + lc
            p = jnp.concatenate([pn[x * 8:x * 8 + 8] for x in reversed(_order(j, _n_vpu(j, c) == 3))], axis=0)
            a = jnp.dot(vtp_ref[j, :, pl.ds(c * CK, CK)], p, preferred_element_type=f32)
            st['acc'][j] = (zero_ref[...] if c == 0 else st['acc'][j]) + a

        def upto(j, gc):
            t, c = divmod(gc, NC)
            return t * per + (first[j][c] + 1) // 2

        done = [upto(j, 1) for j in range(J)]
        for j in range(J):
            mxu_probs(j, 0, done[j])
        for t in range(UN):
            for c in range(NC):
                for j in range(J):
                    need = min(UN * per, upto(j, t * NC + c + 2) + _OFF[j])
                    mxu_probs(j, done[j], need)
                    done[j] = need
                p2 = vpu_probs(t, tuple(range(J)), c * 24 + 8, 16)
                p1 = vpu_probs(t, _EXTRA[c % len(_EXTRA)], c * 24, 8)
                for j in range(J):
                    ps = prows.pop((t, c, j)) + ([p1[j]] if j in p1 else []) + [p2[j]]
                    pv(t, c, j, jnp.concatenate(ps, axis=0))
                if c == NC - 1:
                    finish(t)
        return 0

    for cp in late_copies:
        cp.start()
    jax.lax.fori_loop(0, NU // UN, fast, 0)

    lall = l_ref[...]
    l_ok = jnp.logical_and(lall >= _L_MIN, lall <= _L_MAX)
    n_bad = jnp.sum(jnp.where(l_ok, 0.0, 1.0))
    safe = jnp.logical_and(n_bad == 0.0, vmax <= _V_MAX)

    @pl.when(jnp.logical_not(safe))
    def _():
        def exact(u, _):
            h, cs = u % H, q_cols(u // H)
            s = jnp.dot(kf_ref[...].astype(bf16)[:, :Dh], qt_ref[head_rows(h), cs], preferred_element_type=f32)
            m = jnp.max(s, axis=0, keepdims=True)
            p = jnp.exp2(s - m)
            l_ref[pl.ds(h, 1), cs] = jnp.sum(p, axis=0, keepdims=True)
            acc_ref[head_rows(h), cs] = jnp.dot(kvt_ref[pl.ds(Dh, Dh), :], p.astype(bf16),
                                                preferred_element_type=f32)
            return 0

        jax.lax.fori_loop(0, NU, exact, 0)

    for cp in late_copies:
        cp.wait()

    def out_copy(i):
        return pltpu.make_async_copy(out_ref.at[q_cols(i), :], o_hbm.at[q_cols(i), :], out_sems.at[i])

    def tail(i, _):
        rs = q_cols(i)
        hmid = jax.lax.dot_general(xn_ref[rs, :], w1t_ref[...], nt, preferred_element_type=f32)
        hmid = (hmid * jax.nn.sigmoid(hmid)).astype(bf16)
        rinv = 1.0 / l_ref[:, rs]
        ot = (acc_ref[:, rs].reshape(H, Dh, TQ) * rinv[:, None, :]).reshape(D, TQ).astype(bf16)
        attn = jax.lax.dot_general(ot, wo_ref[...], (((0,), (0,)), ((), ())), preferred_element_type=f32)
        ffn = jnp.dot(hmid, w2_ref[...], preferred_element_type=f32)
        out_ref[rs, :] = (x_ref[rs, :].astype(f32) + attn + ffn).astype(out_ref.dtype)
        out_copy(i).start()
        return 0

    jax.lax.fori_loop(0, NQ, tail, 0)
    for i in range(NQ):
        out_copy(i).wait()


@jax.jit
def pallas_parallel_sum__grouped_kv_mqa__dense_activation_silu__prompt_kernel(
    A_x: jax.Array,
    A_wq: jax.Array,
    A_wk: jax.Array,
    A_wv: jax.Array,
    A_wo: jax.Array,
    B_x: jax.Array,
    B_w1: jax.Array,
    B_w2: jax.Array,
):
    del B_x
    B, S, D = A_x.shape
    assert B == 1
    F = B_w1.shape[1]
    Dh = D // _H
    NC, NQ = S // _CK, S // _TQ
    n_mxu = sum(_NH - _n_vpu(0, c) for c in range(NC))
    x = A_x.reshape(S, D)
    bf16, f32, u32 = jnp.bfloat16, jnp.float32, jnp.uint32
    hbm = pl.BlockSpec(memory_space=pl.ANY)

    out = pl.pallas_call(
        functools.partial(_kernel, S=S, D=D, Dh=Dh),
        out_shape=jax.ShapeDtypeStruct((S, D), A_x.dtype),
        in_specs=[hbm] * 7,
        out_specs=hbm,
        scratch_shapes=[
            pltpu.VMEM((S, D), bf16),
            pltpu.VMEM((D, D), bf16),
            pltpu.VMEM((D, D), bf16),
            pltpu.VMEM((F, D), bf16),
            pltpu.VMEM((F, D), bf16),
            pltpu.VMEM((S, D), A_x.dtype),
            pltpu.VMEM((S, D), bf16),
            pltpu.VMEM((D + 2 * Dh, D), bf16),
            pltpu.VMEM((D, S), bf16),
            pltpu.VMEM((2 * Dh, S), bf16),
            pltpu.VMEM((S, 128), f32),
            pltpu.VMEM((len(_EXTRA), n_mxu * 4, 128), u32),
            pltpu.VMEM((_CK // 2, 128), u32),
            pltpu.VMEM((Dh, NC * 24, 128), f32),
            pltpu.VMEM((_J, Dh, S), f32),
            pltpu.VMEM((_UN, Dh, _TQ), f32),
            pltpu.VMEM((D, S), f32),
            pltpu.VMEM((_H, S), f32),
            pltpu.VMEM((Dh, 128), f32),
            pltpu.SemaphoreType.DMA((NQ + 6,)),
            pltpu.SemaphoreType.DMA((NQ,)),
        ],
        compiler_params=pltpu.CompilerParams(vmem_limit_bytes=100 * 1024 * 1024),
    )(x, A_wq, A_wk.T, A_wv.T, A_wo, B_w1.T, B_w2)
    return out.reshape(B, S, D)
```

```python
import functools
import math

import jax
import jax.numpy as jnp
import jax.experimental.pallas as pl
import jax.experimental.pallas.tpu as pltpu

_H = 32
_EPS = 1e-5
_TQ = 512
_J = _TQ // 128
_CK = 128
_NH = _CK // 8
_UN = 16

_EXTRA = ((0, 1), (2, 3))
_POS = (0, 5, 7, 13)
_XP = (13, 11, 9, 9)
_OFF = (2, 1, 1, 1)

_L_MIN = 2.0 ** -30
_L_MAX = 2.0 ** 100
_V_MAX = 2.0 ** 20


def _n_vpu(j, c):
    return 3 if j in _EXTRA[c % len(_EXTRA)] else 2


def _order(j, extra):
    o = list(range(_NH - 3 if extra else _NH - 2))
    if extra:
        o.insert(min(_XP[j], len(o)), _NH - 3)
    p = min(_POS[j], len(o))
    o[p:p] = [_NH - 2, _NH - 1]
    return o


def _kernel(x_hbm, wq_hbm, wkt_hbm, wvt_hbm, wo_hbm, w1t_hbm, w2_hbm, o_hbm,
            x_ref, wq_ref, wo_ref, w1t_ref, w2_ref, out_ref,
            xn_ref, wqt_ref, qt_ref, kvt_ref, kf_ref, km_ref, km2_ref, kb_ref, vtp_ref,
            qs_ref, acc_ref, l_ref, zero_ref, in_sems, out_sems, *, S, D, Dh):
    f32, bf16, u32 = jnp.float32, jnp.bfloat16, jnp.uint32
    H, TQ, J, CK, NH, UN = _H, _TQ, _J, _CK, _NH, _UN
    NQ, NC = S // TQ, S // CK
    NU, CPT = NQ * H, TQ // CK
    qscale = (Dh ** -0.5) * math.log2(math.e)
    nt = (((1,), (1,)), ((), ()))

    stream = [[(c, x) for c in range(NC) for x in range(NH - _n_vpu(j, c))] for j in range(J)]
    first = [[sum(NH - _n_vpu(j, cc) for cc in range(c)) for c in range(NC + 1)] for j in range(J)]
    per = len(stream[0]) // 2

    def x_copy(i):
        return pltpu.make_async_copy(x_hbm.at[pl.ds(i * TQ, TQ), :], x_ref.at[pl.ds(i * TQ, TQ), :],
                                     in_sems.at[i])

    wq_copy = pltpu.make_async_copy(wq_hbm, wq_ref, in_sems.at[NQ])
    wk_copy = pltpu.make_async_copy(wkt_hbm, wqt_ref.at[pl.ds(D, Dh), :], in_sems.at[NQ + 1])
    wv_copy = pltpu.make_async_copy(wvt_hbm, wqt_ref.at[pl.ds(D + Dh, Dh), :], in_sems.at[NQ + 2])
    late_copies = [pltpu.make_async_copy(src, dst, in_sems.at[NQ + 3 + n])
                   for n, (src, dst) in enumerate([(wo_hbm, wo_ref), (w1t_hbm, w1t_ref), (w2_hbm, w2_ref)])]
    wk_copy.start()
    wv_copy.start()
    wq_copy.start()
    x_copy(0).start()

    def layernorm(i):
        x = x_ref[pl.ds(i * TQ, TQ), :].astype(f32)
        mu = jnp.mean(x, axis=-1, keepdims=True)
        xc = x - mu
        var = jnp.mean(xc * xc, axis=-1, keepdims=True)
        xn_ref[pl.ds(i * TQ, TQ), :] = (xc * jax.lax.rsqrt(var + _EPS)).astype(bf16)

    def project_a(i):
        xn = xn_ref[pl.ds(i * TQ, TQ), :]
        r = jax.lax.dot_general(wqt_ref[pl.ds(D // 2, D // 2 + 2 * Dh), :], xn, nt, preferred_element_type=f32)
        qt_ref[pl.ds(D // 2, D // 2), pl.ds(i * TQ, TQ)] = (r[:D // 2] * qscale).astype(bf16)
        kvt_ref[:, pl.ds(i * TQ, TQ)] = r[D // 2:].astype(bf16)

    def project_b(i):
        xn = xn_ref[pl.ds(i * TQ, TQ), :]
        r = jax.lax.dot_general(wqt_ref[pl.ds(0, D // 2), :], xn, nt, preferred_element_type=f32)
        qt_ref[pl.ds(0, D // 2), pl.ds(i * TQ, TQ)] = (r * qscale).astype(bf16)

    src_key = jax.lax.broadcasted_iota(jnp.int32, (CK, CK), 0)
    dst_key = jax.lax.broadcasted_iota(jnp.int32, (CK, CK), 1)
    dst_row = jax.lax.broadcasted_iota(jnp.int32, (1, CK), 1)

    def perm(j, extra):
        halves = list(reversed(_order(j, extra)))
        want = jnp.zeros((1, CK), jnp.int32)
        for slot, x in enumerate(halves):
            want = jnp.where(dst_row // 8 == slot, x * 8 + dst_row % 8, want)
        return (src_key == want).astype(bf16)

    perms = [[perm(j, extra) for extra in (False, True)] for j in range(J)]

    def tables(i):
        kvt = kvt_ref[:, pl.ds(i * TQ, TQ)]
        vts = [kvt[Dh:, n * CK:(n + 1) * CK] for n in range(CPT)]
        for j in range(J):
            for extra in (False, True):
                ns = [n for n in range(CPT) if (_n_vpu(j, i * CPT + n) == 3) == extra]
                if not ns:
                    continue
                vp = jnp.dot(jnp.concatenate([vts[n] for n in ns], axis=0), perms[j][extra],
                             preferred_element_type=f32)
                for r, n in enumerate(ns):
                    vtp_ref[j, :, pl.ds((i * CPT + n) * CK, CK)] = vp[r * Dh:(r + 1) * Dh, :]
        kt = kvt[:Dh].astype(f32)
        knat = jnp.concatenate([kt, jnp.zeros((128 - Dh, TQ), f32)], axis=0).T
        kf_ref[pl.ds(i * TQ, TQ), :] = knat
        for n in range(CPT):
            kv = knat[(n + 1) * CK - 24:(n + 1) * CK, :]
            for d in range(Dh):
                kb_ref[d, pl.ds((i * CPT + n) * 24, 24), :] = jnp.broadcast_to(kv[:, d:d + 1], (24, 128))
        if i % 2 == 1:
            c0, c1 = (i - 1) * CPT, (i + 1) * CPT
            for j in range(J):
                rows = jnp.concatenate([kf_ref[pl.ds(c * CK, 8 * (NH - _n_vpu(j, c))), :]
                                        for c in range(c0, c1)], axis=0)
                km_ref[j, pl.ds(first[j][c0] * 4, (first[j][c1] - first[j][c0]) * 4), :] = pltpu.bitcast(
                    rows.astype(bf16), u32)
        if i == 0:
            ksh = jnp.concatenate([jnp.zeros((Dh, CK), f32), kt[:, :CK],
                                   jnp.zeros((128 - 2 * Dh, CK), f32)], axis=0).T
            km2_ref[...] = pltpu.bitcast(ksh.astype(bf16), u32)

    zero_ref[...] = jnp.zeros(zero_ref.shape, f32)
    wk_copy.wait()
    wv_copy.wait()
    wq_copy.wait()
    eye = (src_key == dst_key).astype(bf16)
    for a in reversed(range(D // CK)):
        wqt_ref[pl.ds(a * CK, CK), :] = jax.lax.dot_general(
            eye, wq_ref[:, pl.ds(a * CK, CK)], nt, preferred_element_type=f32).astype(bf16)
    x_copy(0).wait()
    for i in range(1, NQ):
        x_copy(i).start()
    for i in range(NQ):
        if i > 0:
            if i < NQ - 1:
                x_copy(i).wait()
            if i == NQ - 2:
                x_copy(i + 1).wait()
            project_b(i - 1)
            tables(i - 1)
        layernorm(i)
        project_a(i)
    project_b(NQ - 1)
    tables(NQ - 1)
    vmax = jnp.max(jnp.abs(kvt_ref[pl.ds(Dh, Dh), :].astype(f32)))

    def head_rows(h):
        return pl.ds(pl.multiple_of(h * Dh, Dh), Dh)

    def q_cols(j):
        return pl.ds(pl.multiple_of(j * TQ, TQ), TQ)

    def fast(i, _):
        sts, qts, qbs, kbs, prows = {}, {}, {}, {}, {}
        h0, cs = (i * UN) % H, q_cols((i * UN) // H)

        def get_q(t):
            if t not in qts:
                qts[t] = qt_ref[head_rows(h0 + t), cs]
                qs_ref[t] = qts[t].astype(f32)
                sts[t] = dict(l=[None] * J, acc=[None] * J)
            return qts[t]

        def finish(t):
            l_ref[pl.ds(h0 + t, 1), cs] = jnp.sum(jnp.concatenate(sts[t]['l'], axis=1), axis=0, keepdims=True)
            acc_ref[head_rows(h0 + t), cs] = jnp.concatenate(sts[t]['acc'], axis=1)

        def mxu_probs(j, a, b):
            if a >= b:
                return
            t0, t1 = a // per, (b - 1) // per
            la = a - t0 * per
            if t0 == t1:
                kk = km_ref[j, pl.ds(la * 8, (b - a) * 8), :]
                kk, w = pltpu.bitcast(kk, bf16)[:, :Dh], get_q(t0)
            else:
                kk = jnp.concatenate([km_ref[j, pl.ds(la * 8, (per - la) * 8), :],
                                      km2_ref[pl.ds(0, (b - t1 * per) * 8), :]], axis=0)
                kk = pltpu.bitcast(kk, bf16)[:, :2 * Dh]
                w = jnp.concatenate([get_q(t0), get_q(t1)], axis=0)
            p = jnp.exp2(jnp.dot(kk, w[:, j * 128:(j + 1) * 128], preferred_element_type=f32))
            x = 2 * a
            while x < 2 * b:
                t, lx = divmod(x, 2 * per)
                c = stream[j][lx][0]
                e = min(2 * b, t * 2 * per + first[j][c + 1])
                prows.setdefault((t, c, j), []).append(p[(x - 2 * a) * 8:(e - 2 * a) * 8, :])
                x = e

        def vpu_probs(t, js, row, n):
            if (row, n) not in kbs:
                kb = kb_ref[:, pl.ds(row, n), :]
                kb = jnp.concatenate([kb] * len(js), axis=2)
                kbs[(row, n)] = [kb[d] for d in range(Dh)]
            acc = None
            for d in range(Dh):
                if (t, d, js) not in qbs:
                    qbs[(t, d, js)] = jnp.concatenate([
                        jnp.broadcast_to(qs_ref[t, pl.ds(d, 1), pl.ds(j * 128, 128)], (n, 128)) for j in js], axis=1)
                y = kbs[(row, n)][d] * qbs[(t, d, js)]
                acc = y if d == 0 else acc + y
            p = jnp.exp2(acc)
            return {j: p[:, k * 128:(k + 1) * 128] for k, j in enumerate(js)}

        def pv(t, c, j, pn):
            st = sts[t]
            lc = jnp.sum(pn.reshape(NH, 8, 128), axis=0)
            st['l'][j] = lc if c == 0 else st['l'][j] + lc
            p = jnp.concatenate([pn[x * 8:x * 8 + 8] for x in reversed(_order(j, _n_vpu(j, c) == 3))], axis=0)
            a = jnp.dot(vtp_ref[j, :, pl.ds(c * CK, CK)], p, precision=jax.lax.Precision.DEFAULT,
                        preferred_element_type=f32)
            st['acc'][j] = (zero_ref[...] if c == 0 else st['acc'][j]) + a

        def upto(j, gc):
            t, c = divmod(gc, NC)
            return t * per + (first[j][c] + 1) // 2

        done = [upto(j, 1) for j in range(J)]
        for j in range(J):
            mxu_probs(j, 0, done[j])
        for t in range(UN):
            for c in range(NC):
                for j in range(J):
                    need = min(UN * per, upto(j, t * NC + c + 2) + _OFF[j])
                    mxu_probs(j, done[j], need)
                    done[j] = need
                p2 = vpu_probs(t, tuple(range(J)), c * 24 + 8, 16)
                p1 = vpu_probs(t, _EXTRA[c % len(_EXTRA)], c * 24, 8)
                for j in range(J):
                    ps = prows.pop((t, c, j)) + ([p1[j]] if j in p1 else []) + [p2[j]]
                    pv(t, c, j, jnp.concatenate(ps, axis=0))
                if c == NC - 1:
                    finish(t)
        return 0

    for cp in late_copies:
        cp.start()
    jax.lax.fori_loop(0, NU // UN, fast, 0)

    lall = l_ref[...]
    l_ok = jnp.logical_and(lall >= _L_MIN, lall <= _L_MAX)
    n_bad = jnp.sum(jnp.where(l_ok, 0.0, 1.0))
    safe = jnp.logical_and(n_bad == 0.0, vmax <= _V_MAX)

    @pl.when(jnp.logical_not(safe))
    def _():
        def exact(u, _):
            h, cs = u % H, q_cols(u // H)
            s = jnp.dot(kf_ref[...].astype(bf16)[:, :Dh], qt_ref[head_rows(h), cs], preferred_element_type=f32)
            m = jnp.max(s, axis=0, keepdims=True)
            p = jnp.exp2(s - m)
            l_ref[pl.ds(h, 1), cs] = jnp.sum(p, axis=0, keepdims=True)
            acc_ref[head_rows(h), cs] = jnp.dot(kvt_ref[pl.ds(Dh, Dh), :], p.astype(bf16),
                                                preferred_element_type=f32)
            return 0

        jax.lax.fori_loop(0, NU, exact, 0)

    for cp in late_copies:
        cp.wait()

    def out_copy(i):
        return pltpu.make_async_copy(out_ref.at[q_cols(i), :], o_hbm.at[q_cols(i), :], out_sems.at[i])

    def tail(i, _):
        rs = q_cols(i)
        hmid = jax.lax.dot_general(xn_ref[rs, :], w1t_ref[...], nt, preferred_element_type=f32)
        hmid = (hmid * jax.nn.sigmoid(hmid)).astype(bf16)
        rinv = 1.0 / l_ref[:, rs]
        ot = (acc_ref[:, rs].reshape(H, Dh, TQ) * rinv[:, None, :]).reshape(D, TQ).astype(bf16)
        attn = jax.lax.dot_general(ot, wo_ref[...], (((0,), (0,)), ((), ())), preferred_element_type=f32)
        ffn = jnp.dot(hmid, w2_ref[...], preferred_element_type=f32)
        out_ref[rs, :] = (x_ref[rs, :].astype(f32) + attn + ffn).astype(out_ref.dtype)
        out_copy(i).start()
        return 0

    jax.lax.fori_loop(0, NQ, tail, 0)
    for i in range(NQ):
        out_copy(i).wait()


@jax.jit
def pallas_parallel_sum__grouped_kv_mqa__dense_activation_silu__prompt_kernel(
    A_x: jax.Array,
    A_wq: jax.Array,
    A_wk: jax.Array,
    A_wv: jax.Array,
    A_wo: jax.Array,
    B_x: jax.Array,
    B_w1: jax.Array,
    B_w2: jax.Array,
):
    del B_x
    B, S, D = A_x.shape
    assert B == 1
    F = B_w1.shape[1]
    Dh = D // _H
    NC, NQ = S // _CK, S // _TQ
    n_mxu = sum(_NH - _n_vpu(0, c) for c in range(NC))
    x = A_x.reshape(S, D)
    bf16, f32, u32 = jnp.bfloat16, jnp.float32, jnp.uint32
    hbm = pl.BlockSpec(memory_space=pl.ANY)

    out = pl.pallas_call(
        functools.partial(_kernel, S=S, D=D, Dh=Dh),
        out_shape=jax.ShapeDtypeStruct((S, D), A_x.dtype),
        in_specs=[hbm] * 7,
        out_specs=hbm,
        scratch_shapes=[
            pltpu.VMEM((S, D), bf16),
            pltpu.VMEM((D, D), bf16),
            pltpu.VMEM((D, D), bf16),
            pltpu.VMEM((F, D), bf16),
            pltpu.VMEM((F, D), bf16),
            pltpu.VMEM((S, D), A_x.dtype),
            pltpu.VMEM((S, D), bf16),
            pltpu.VMEM((D + 2 * Dh, D), bf16),
            pltpu.VMEM((D, S), bf16),
            pltpu.VMEM((2 * Dh, S), bf16),
            pltpu.VMEM((S, 128), f32),
            pltpu.VMEM((_J, n_mxu * 4, 128), u32),
            pltpu.VMEM((_CK // 2, 128), u32),
            pltpu.VMEM((Dh, NC * 24, 128), f32),
            pltpu.VMEM((_J, Dh, S), f32),
            pltpu.VMEM((_UN, Dh, _TQ), f32),
            pltpu.VMEM((D, S), f32),
            pltpu.VMEM((_H, S), f32),
            pltpu.VMEM((Dh, 128), f32),
            pltpu.SemaphoreType.DMA((NQ + 6,)),
            pltpu.SemaphoreType.DMA((NQ,)),
        ],
        compiler_params=pltpu.CompilerParams(vmem_limit_bytes=100 * 1024 * 1024),
    )(x, A_wq, A_wk.T, A_wv.T, A_wo, B_w1.T, B_w2)
    return out.reshape(B, S, D)
```
